```python
import jax
import jax.numpy as jnp

def _softmax(x, axis=-1):
    return jax.nn.softmax(x, axis=axis)
def _gelu(x):
    return jax.nn.gelu(x, approximate=True)
def _silu(x):
    return jax.nn.silu(x)
def _sigmoid(x):
    return jax.nn.sigmoid(x)
def _layernorm(x, axis=-1, eps=1e-5):
    m = jnp.mean(x, axis=axis, keepdims=True)
    v = jnp.var(x, axis=axis, keepdims=True)
    return (x - m) / jnp.sqrt(v + eps)
def _scatter_add(tgt, idx, src, axis=0):
    return tgt.at[idx].add(src)
def _segment_sum(src, seg, n):
    return jax.ops.segment_sum(src, seg, n)
class _Rng:
    def __init__(self, key):
        self._k = key
    def _next(self):
        self._k, sub = jax.random.split(self._k)
        return sub
    def normal(self, shape):
        return jax.random.normal(self._next(), shape, dtype=jnp.bfloat16)
    def randint(self, lo, hi, shape):
        return jax.random.randint(self._next(), shape, lo, hi, dtype=jnp.int32)
    def uniform(self, shape, lo=0.0, hi=1.0):
        return jax.random.uniform(self._next(), shape, jnp.bfloat16, lo, hi)
    def permutation(self, n):
        return jax.random.permutation(self._next(), n)


kernel_name = 'interleave_layers__sliding_block_cached__glu_gated_glu__decode'

def setup_inputs():
    _rng = _Rng(jax.random.key(int.from_bytes(__import__("os").urandom(4), "little")))
    _w = (lambda a: (lambda t: t.astype(jnp.bfloat16) if jnp.issubdtype(t.dtype, jnp.floating) else t)(jnp.asarray(a)))
    def _A_setup():
        B, Sq, D = 1, 1, 640
        Hq, Hkv, Sk, Dh = 32, 32, 32768, 192
        assert Hq % Hkv == 0, (Hq, Hkv)
        return {
            "x": _w((lambda *s: _rng.normal(s) * 0.05)(B, Sq, D)),
            "k_cache": _w((lambda *s: _rng.normal(s) * 0.05)(B, Hkv, Sk, Dh)),
            "v_cache": _w((lambda *s: _rng.normal(s) * 0.05)(B, Hkv, Sk, Dh)),
            "wq": _w((lambda *s: _rng.normal(s) * 0.05)(D, Hq * Dh) * (D ** -0.5)),
            "wo": _w((lambda *s: _rng.normal(s) * 0.05)(Hq * Dh, D) * ((Hq * Dh) ** -0.5)),
        }
    _A_in = _A_setup()

    def _B_setup():
        B, S, D, F = 1, 1, 640, 1536
        return {
            "x": _w((lambda *s: _rng.normal(s) * 0.05)(B, S, D)),
            "w_gate": _w((lambda *s: _rng.normal(s) * 0.05)(D, F)),
            "w_up": _w((lambda *s: _rng.normal(s) * 0.05)(D, F)),
            "w_down": _w((lambda *s: _rng.normal(s) * 0.05)(F, D)),
        }
    _B_in = _B_setup()

    return {
        "A_x": _A_in["x"],
        "A_k_cache": _A_in["k_cache"],
        "A_v_cache": _A_in["v_cache"],
        "A_wq": _A_in["wq"],
        "A_wo": _A_in["wo"],
        "B_x": _B_in["x"],
        "B_w_gate": _B_in["w_gate"],
        "B_w_up": _B_in["w_up"],
        "B_w_down": _B_in["w_down"],
    }

def reference(A_x, A_k_cache, A_v_cache, A_wq, A_wo, B_x, B_w_gate, B_w_up, B_w_down):
    def _A_ref(x, k_cache, v_cache, wq, wo):
        B, Sq, D = x.shape
        Hq, Dh = 32, 192
        Hkv, Sk = k_cache.shape[1], k_cache.shape[2]
        W = min(4096, max(256, Sk // 4))
        rep = Hq // Hkv
        q = (lambda x, *d: x.transpose(*d))((x @ wq).reshape(B, Sq, Hq, Dh), 0, 2, 1, 3)
        k = jnp.repeat(k_cache[:, :, Sk - W:, :], rep, axis=1)
        v = jnp.repeat(v_cache[:, :, Sk - W:, :], rep, axis=1)
        scores = jnp.einsum("bhqd,bhkd->bhqk", q, k) * (Dh ** -0.5)
        p = _softmax(scores, axis=-1)
        o = jnp.einsum("bhqk,bhkd->bhqd", p, v)
        return (lambda x, *d: x.transpose(*d))(o, 0, 2, 1, 3).reshape(B, Sq, Hq * Dh) @ wo

    def _B_ref(x, w_gate, w_up, w_down):
        g = jnp.einsum("bsd,df->bsf", x, w_gate)
        u = jnp.einsum("bsd,df->bsf", x, w_up)
        h = _sigmoid(g) * u
        return jnp.einsum("bsf,fd->bsd", h, w_down)

    x = A_x
    x = x + _A_ref(_layernorm(x, axis=-1), A_k_cache, A_v_cache, A_wq, A_wo)
    x = x + _B_ref(_layernorm(x, axis=-1), B_w_gate, B_w_up, B_w_down)
    x = x + _A_ref(_layernorm(x, axis=-1), A_k_cache, A_v_cache, A_wq, A_wo)
    x = x + _B_ref(_layernorm(x, axis=-1), B_w_gate, B_w_up, B_w_down)
    return x
```

```python
import jax
import jax.numpy as jnp
from jax import lax
import jax.experimental.pallas as pl
import jax.experimental.pallas.tpu as pltpu

F32 = jnp.float32
BF16 = jnp.bfloat16
U32 = jnp.uint32

HQ, DH = 32, 192
NA = DH // 8
CH = 128
EPS = 1e-5
WD_PIECES = ((0, 6), (6, 10), (10, 11), (11, 12))


def _tile_view(w):
    *lead, r, c = w.shape
    n = len(lead)
    t = w.reshape(*lead, r // 8, 8, c // 128, 128)
    t = jnp.transpose(t, (*range(n), n, n + 2, n + 1, n + 3))
    return t.reshape(*lead, r // 8, c // 128 * 8, 128)


def _interleave(*gens):
    live = [list(g) for g in gens]
    while live:
        for item in list(live):
            for _ in range(item[1]):
                try:
                    next(item[0])
                except StopIteration:
                    live.remove(item)
                    break


def _drain(gen):
    for _ in gen:
        pass


def _make_kernel(d_model, d_ff, sk, win):
    NB = win // 256
    HR = NA * NB * 16
    WIN0 = (sk - win) // 16
    ND = d_model // 128
    NF = d_ff // 128
    NQ = HQ * DH // 128
    WO_ROWS = 2 * NA * ND * 8
    S_K, S_V, S_O = 0, HQ, 2 * HQ
    S_Q = S_O + HQ // 2
    NSQ = 5
    S_G, S_U, S_X, S_D = S_Q + NSQ, S_Q + NSQ + 1, S_Q + NSQ + 2, S_Q + NSQ + 3
    n_sems = S_D + len(WD_PIECES)

    def kernel(x_hbm, k_hbm, v_hbm, wq_hbm, wo_hbm, wg_hbm, wu_hbm, wd_hbm, o_ref,
               xb, kb, vb, wq, wo, wg, wu, wd, lx, lq, pb, ab, yb, sems):
        lane = lax.broadcasted_iota(jnp.int32, (8, 128), 1)
        sub = lax.broadcasted_iota(jnp.int32, (8, 128), 0)
        lane_c = (lane >> 3) & 1
        spread = ((lane >> 4) << 3) | (lane & 7)

        def start_rows(src, dst, row0, nrows, sem):
            def pair(j, _):
                for p in range(2):
                    r = pl.multiple_of(row0 + (2 * j + p) * CH, CH)
                    pltpu.make_async_copy(src.at[pl.ds(r, CH)], dst.at[pl.ds(r, CH)],
                                          sems.at[sem]).start(priority=p)
            n = nrows // CH
            lax.fori_loop(0, n // 2, pair, None)
            if n % 2:
                r = pl.multiple_of(row0 + (n - 1) * CH, CH)
                pltpu.make_async_copy(src.at[pl.ds(r, CH)], dst.at[pl.ds(r, CH)],
                                      sems.at[sem]).start()

        def wait_rows(dst, row0, nrows, sem):
            blk = dst.at[pl.ds(row0, nrows)]
            pltpu.make_async_copy(blk, blk, sems.at[sem]).wait()

        def start_head(src, dst, h, sem):
            def group(a, _):
                for p in range(NB * 16 // CH):
                    r = pl.multiple_of(a * (NB * 16) + p * CH, CH)
                    pltpu.make_async_copy(src.at[h * NA + a, pl.ds(WIN0 + p * CH, CH)],
                                          dst.at[h, pl.ds(r, CH)],
                                          sems.at[sem]).start(priority=p % 2)
            lax.fori_loop(0, NA, group, None, unroll=4)

        def wait_head(dst, h, sem):
            pltpu.make_async_copy(dst.at[h], dst.at[h], sems.at[sem]).wait()

        def vregs(pieces):
            cols = [jnp.concatenate([pltpu.bitcast(p, U32) for p in col], axis=0)
                    for col in pieces]
            return pltpu.bitcast(jnp.concatenate(cols, axis=1), BF16)

        def mm(lhs, rhs):
            return jnp.dot(lhs, rhs, preferred_element_type=F32)

        def pack(lo, hi):
            return jnp.concatenate([lo, hi], axis=0).astype(BF16)

        def halves(t):
            return [jnp.take_along_axis(t, spread + off, axis=1) for off in (0, 64)]

        def layernorm_lhs(x):
            m = jnp.sum(x, axis=1, keepdims=True) * (1.0 / d_model)
            xc = x - m
            v = jnp.sum(xc * xc, axis=1, keepdims=True) * (1.0 / d_model)
            rs = lax.rsqrt(v + EPS)
            for t in range(ND):
                for j, g in enumerate(halves(x[:, t * 128:(t + 1) * 128])):
                    n = (g - m) * rs
                    i = 2 * t + j
                    lx[i * 16:(i + 1) * 16, :] = pack(jnp.where(lane_c == 0, n, 0.0),
                                                      jnp.where(lane_c == 1, n, 0.0))

        def x_matmul(w, ntiles, cp):
            acc = None
            for i in range(2 * ND):
                col = [w[pl.ds(pl.multiple_of((8 * i + a) * ntiles * 8 + cp * 16, 16), 16), :]
                       for a in range(8)]
                r = mm(lx[i * 16:(i + 1) * 16, :], vregs([col]))
                acc = r if acc is None else acc + r
            return acc[0:8], acc[8:16]

        def q_tiles(cp):
            for c, t in enumerate(x_matmul(wq, NQ, cp)):
                for j, g in enumerate(halves(t)):
                    g = jnp.where(lane_c == (sub & 1), g, 0.0)
                    r = pl.multiple_of((4 * cp + 2 * c + j) * 16, 16)
                    lq[pl.ds(r, 16), :] = pack(g, g)

        def scores_softmax(h, slot):
            q = jnp.concatenate(
                [lq[pl.ds(pl.multiple_of((3 * h + t) * 16, 16), 16), :] for t in range(NA // 8)],
                axis=1)
            parts = []
            for g in range(NB // 4):
                s = None
                for j in range(4):
                    b = 4 * g + j
                    col = [kb[h, (a * NB + b) * 16:(a * NB + b + 1) * 16, :] for a in range(NA)]
                    r = mm(q, vregs([col]))[0:8]
                    s = r if s is None else jnp.where((sub >> 1) == j, r, s)
                    yield
                parts.append(s)
            s = jnp.concatenate(parts, axis=0)
            m = jnp.max(jnp.max(s, axis=0, keepdims=True), axis=1, keepdims=True)
            e = jnp.exp((s - m) * (DH ** -0.5))
            den = jnp.sum(jnp.sum(e, axis=0, keepdims=True), axis=1, keepdims=True)
            p = e * (1.0 / den)
            for i in range(2 * NB):
                pb[slot, i * 8:(i + 1) * 8, :] = jnp.broadcast_to(p[i:i + 1, :], (8, 128))

        def p_times_v(h, slot, row0):
            for a0 in range(0, NA, 8):
                acc = [None] * 8
                for b in range(NB):
                    p0 = pb[slot, b * 16:b * 16 + 8, :]
                    p1 = pb[slot, b * 16 + 8:b * 16 + 16, :]
                    for i in range(8):
                        r = ((a0 + i) * NB + b) * 16
                        v = vb[h, r:r + 16, :].astype(F32)
                        t = v[0:8] * p0 + v[8:16] * p1
                        acc[i] = t if acc[i] is None else acc[i] + t
                    yield
                for i in range(8):
                    ab[pl.ds(pl.multiple_of(row0 + (a0 + i) * 8, 8), 8), :] = acc[i]

        def retile(w, g0, n):
            def body(g, _):
                r = pl.multiple_of((g0 + g) * (ND * 16), 16)
                new = [jnp.concatenate([w[pl.ds(r + t * 8, 8), :],
                                        w[pl.ds(r + (ND + t) * 8, 8), :]], axis=0)
                       for t in range(ND)]
                for t in range(ND):
                    w[pl.ds(r + t * 16, 16), :] = new[t]
            lax.fori_loop(0, n, body, None, unroll=4)

        def row_matmul(lhs, w, g0):
            cols = [[w[pl.ds(pl.multiple_of(((g0 + g) * ND + t) * 16, 16), 16), :]
                     for g in range(8)] for t in range(ND)]
            return mm(lhs, vregs(cols))[0:8]

        def out_proj(pair, row0):
            y = None
            for j in range(2 * DH // 128):
                o = jnp.sum(ab[row0 + j * 128:row0 + (j + 1) * 128, :].T, axis=0, keepdims=True)
                lhs = jnp.broadcast_to(o, (16, 128)).astype(BF16)
                r = row_matmul(lhs, wo, pair * NA + j * 8)
                y = r if y is None else y + r
            return y

        def residual(x, y):
            return (x + y.astype(BF16).astype(F32)).astype(BF16).astype(F32)

        def glu_hidden(g, u):
            hid = jax.nn.sigmoid(g) * u
            return pack(hid, hid)

        wq_step = d_model * NQ // NSQ
        start_rows(wq_hbm, wq, 0, wq_step, S_Q)
        x_copy = pltpu.make_async_copy(x_hbm, xb, sems.at[S_X])
        x_copy.start()
        start_rows(wq_hbm, wq, wq_step, wq_step, S_Q + 1)
        x_copy.wait()
        x = jnp.broadcast_to(xb[...].astype(F32), (8, d_model))
        layernorm_lhs(x)
        yb[...] = jnp.zeros_like(yb)
        for s in range(NSQ):
            wait_rows(wq, s * wq_step, wq_step, S_Q + s)
            if s + 2 < NSQ:
                start_rows(wq_hbm, wq, (s + 2) * wq_step, wq_step, S_Q + s + 2)
            elif s + 2 == NSQ:
                start_head(k_hbm, kb, 0, S_K)
            else:
                start_head(v_hbm, vb, 0, S_V)
        lax.fori_loop(0, NQ // 2, lambda cp, _: q_tiles(cp), None)

        def head1(h, _):
            odd = h & 1
            wait_head(kb, h, S_K + h)

            @pl.when(h + 1 < HQ)
            def _():
                start_head(k_hbm, kb, h + 1, S_K + h + 1)

            @pl.when(h + 1 == HQ)
            def _():
                start_rows(wg_hbm, wg, 0, d_model * NF, S_G)

            _drain(scores_softmax(h, 0))
            wait_head(vb, h, S_V + h)

            @pl.when(h + 1 < HQ)
            def _():
                start_head(v_hbm, vb, h + 1, S_V + h + 1)

            @pl.when(h + 1 == HQ)
            def _():
                start_rows(wu_hbm, wu, 0, d_model * NF, S_U)

            @pl.when(odd == 0)
            def _():
                start_rows(wo_hbm, wo, (h >> 1) * WO_ROWS, WO_ROWS, S_O + (h >> 1))

            _drain(p_times_v(h, 0, odd * DH))

            @pl.when(odd == 1)
            def _():
                pair = h >> 1
                wait_rows(wo, pl.multiple_of(pair * WO_ROWS, CH), WO_ROWS, S_O + pair)
                retile(wo, pair * NA, NA)
                yb[...] += out_proj(pair, 0)

        lax.fori_loop(0, HQ, head1, None)

        for i, (k0, k1) in enumerate(WD_PIECES):
            start_rows(wd_hbm, wd, k0 * 128 * ND, (k1 - k0) * 128 * ND, S_D + i)
        x = residual(x, yb[...])
        layernorm_lhs(x)
        wait_rows(wg, 0, d_model * NF, S_G)
        gate = [t for cp in range(NF // 2) for t in x_matmul(wg, NF, cp)]
        wait_rows(wu, 0, d_model * NF, S_U)
        up = [t for cp in range(NF // 2) for t in x_matmul(wu, NF, cp)]
        hid = [glu_hidden(g, u) for g, u in zip(gate, up)]
        y = None
        for i, (k0, k1) in enumerate(WD_PIECES):
            wait_rows(wd, k0 * 128 * ND, (k1 - k0) * 128 * ND, S_D + i)
            retile(wd, k0 * 8, (k1 - k0) * 8)
            for k in range(k0, k1):
                r = row_matmul(hid[k], wd, k * 8)
                y = r if y is None else y + r
        x = residual(x, y)

        layernorm_lhs(x)
        q_tiles(0)
        q_tiles(1)
        _drain(scores_softmax(0, 0))

        def quad(i, y):
            for k in range(4):
                h = 4 * i + k
                if k < 3:
                    q_tiles(jnp.minimum(3 * i + 2 + k, NQ // 2 - 1))
                if k == 1:
                    prev = out_proj(jnp.maximum(2 * i - 1, 0), 2 * DH)
                    y = y + jnp.where(i > 0, prev, 0.0)
                if k == 3:
                    y = y + out_proj(2 * i, 0)
                _interleave((p_times_v(h, k % 2, k * DH), 3),
                            (scores_softmax(jnp.minimum(h + 1, HQ - 1), (k + 1) % 2), 1))
            return y

        ab[2 * DH:4 * DH, :] = jnp.zeros((2 * DH, 128), F32)
        y = lax.fori_loop(0, HQ // 4, quad, jnp.zeros((8, d_model), F32))
        y = y + out_proj(HQ // 2 - 1, 2 * DH)
        x = residual(x, y)

        layernorm_lhs(x)
        y = None
        for cp in range(NF // 2):
            gate = x_matmul(wg, NF, cp)
            up = x_matmul(wu, NF, cp)
            for c in range(2):
                r = row_matmul(glu_hidden(gate[c], up[c]), wd, (2 * cp + c) * 8)
                y = r if y is None else y + r
        o_ref[...] = residual(x, y)[0:1].astype(o_ref.dtype)

    scratch = [
        pltpu.VMEM((1, d_model), BF16),
        pltpu.VMEM((HQ, HR, 128), BF16),
        pltpu.VMEM((HQ, HR, 128), BF16),
        pltpu.VMEM((d_model * NQ, 128), BF16),
        pltpu.VMEM((HQ * DH * ND, 128), BF16),
        pltpu.VMEM((d_model * NF, 128), BF16),
        pltpu.VMEM((d_model * NF, 128), BF16),
        pltpu.VMEM((d_ff * ND, 128), BF16),
        pltpu.VMEM((2 * ND * 16, 128), BF16),
        pltpu.VMEM((2 * NQ * 16, 128), BF16),
        pltpu.VMEM((2, 2 * NB * 8, 128), F32),
        pltpu.VMEM((4 * DH, 128), F32),
        pltpu.VMEM((8, d_model), F32),
        pltpu.SemaphoreType.DMA((n_sems,)),
    ]
    return kernel, scratch


@jax.jit
def pallas_interleave_layers__sliding_block_cached__glu_gated_glu__decode_kernel(
    A_x: jax.Array,
    A_k_cache: jax.Array,
    A_v_cache: jax.Array,
    A_wq: jax.Array,
    A_wo: jax.Array,
    B_x: jax.Array,
    B_w_gate: jax.Array,
    B_w_up: jax.Array,
    B_w_down: jax.Array,
):
    del B_x
    d_model, d_ff = B_w_gate.shape
    sk = A_k_cache.shape[2]
    win = min(4096, max(256, sk // 4))
    assert A_x.shape == (1, 1, 640) and d_ff == 1536 and win == 4096
    assert A_k_cache.shape == A_v_cache.shape == (1, HQ, sk, DH) and sk % 256 == 0

    def cache_view(c):
        t = jnp.swapaxes(c, 2, 3).reshape(HQ, DH, sk)
        return _tile_view(t).reshape(HQ * NA, sk // 16, 128)

    def weight_view(w):
        return _tile_view(w).reshape(-1, 128)

    kernel, scratch = _make_kernel(d_model, d_ff, sk, win)
    out = pl.pallas_call(
        kernel,
        out_shape=jax.ShapeDtypeStruct((1, d_model), A_x.dtype),
        in_specs=[pl.BlockSpec(memory_space=pl.ANY)] * 8,
        out_specs=pl.BlockSpec(memory_space=pltpu.VMEM),
        scratch_shapes=scratch,
        compiler_params=pltpu.CompilerParams(vmem_limit_bytes=126 * 1024 * 1024),
        name="attn_glu_x2",
    )(A_x.reshape(1, d_model), cache_view(A_k_cache), cache_view(A_v_cache),
      weight_view(A_wq), weight_view(A_wo), weight_view(B_w_gate), weight_view(B_w_up),
      weight_view(B_w_down))
    return out.reshape(A_x.shape)
```

```python
import jax
import jax.numpy as jnp
from jax import lax
import jax.experimental.pallas as pl
import jax.experimental.pallas.tpu as pltpu

F32 = jnp.float32
BF16 = jnp.bfloat16
U32 = jnp.uint32

HQ, DH = 32, 192
NA = DH // 8
CH = 8
EPS = 1e-5
WD_PIECES = ((0, 6), (6, 10), (10, 11), (11, 12))
ACC, MXU_SEGS, DELAY, SM_DELAY, CHAIN = 8, 82, 14, 16, 0


def _vreg_view(w):
    *lead, r, c = w.shape
    n = len(lead)
    t = w.reshape(*lead, r // 8, 8, c // 128, 128)
    t = jnp.transpose(t, (*range(n), n, n + 2, n + 1, n + 3))
    return t.reshape(-1, 16, 128)


def _run(gen):
    try:
        while True:
            next(gen)
    except StopIteration as stop:
        return stop.value


def _make_kernel(d_model, d_ff, sk, win):
    NB = win // 256
    HV = NA * NB
    ND = d_model // 128
    NF = d_ff // 128
    NQ = HQ * DH // 128
    KT = 8 * ND
    NSQ = 5
    S_K, S_V, S_O, S_Q = 0, 1, 2, 3
    S_G, S_U, S_X, S_D = S_K, S_V, S_O, S_Q
    n_sems = S_D + max(2, len(WD_PIECES))
    sizes = dict(k=HQ * HV, v=HQ * HV, wq=NQ * KT, wo=NQ * KT, wg=NF * KT, wu=NF * KT,
                 wd=NF * KT)
    work = dict(p=4 * NB, s=NB // 4, y=ND, r=HQ + 1, q=2 * NQ, x=2 * ND)
    at, total = {}, 0
    for name, size in sizes.items():
        at[name], total = total, total + size

    def kernel(x_hbm, k_hbm, v_hbm, wq_hbm, wo_hbm, wg_hbm, wu_hbm, wd_hbm, o_ref,
               xb, buf, ab, sems, *work_refs):
        wk = dict(zip(work, work_refs))
        lane = lax.broadcasted_iota(jnp.int32, (8, 128), 1)
        sub = lax.broadcasted_iota(jnp.int32, (8, 128), 0)
        lane_c = (lane >> 3) & 1
        spread = ((lane >> 4) << 3) | (lane & 7)

        hbm = dict(k=k_hbm, v=v_hbm, wq=wq_hbm, wo=wo_hbm, wg=wg_hbm, wu=wu_hbm, wd=wd_hbm)
        hbm = {name: ref.bitcast(U32) for name, ref in hbm.items()}

        def piece(name, src, dst, sem, queue):
            pltpu.make_async_copy(hbm[name].at[pl.ds(src, CH)],
                                  buf.at[pl.ds(at[name] + dst, CH)],
                                  sems.at[sem]).start(priority=queue)

        def start(name, i0, n, sem):
            def body(j, _):
                for c in range(2):
                    piece(name, i0 + (2 * j + c) * CH, i0 + (2 * j + c) * CH, sem, c)
            lax.fori_loop(0, n // (2 * CH), body, None)
            if n // CH % 2:
                piece(name, i0 + n - CH, i0 + n - CH, sem, 0)

        def start_head(name, h, sem):
            def body(a, _):
                for c in range(NB // CH):
                    piece(name, (h * NA + a) * (sk // 256) + (sk // 256 - NB + c * CH),
                          (h * NA + a) * NB + c * CH, sem, c % 2)
            lax.fori_loop(0, NA, body, None, unroll=2)

        def wait(name, i0, n, sem):
            blk = buf.at[pl.ds(at[name] + i0, n)]
            pltpu.make_async_copy(blk, blk, sems.at[sem]).wait()

        def load(name, base, off):
            return buf[base + (at[name] + off)] if name in sizes else wk[name][base + off]

        def put(name, base, vals):
            for i, v in enumerate(vals):
                wk[name][base + i] = pltpu.bitcast(v, U32)

        def get(name, base, n, off=0):
            return [pltpu.bitcast(load(name, base, off + i), F32) for i in range(n)]

        def tile_matmul(lhs, rhs):
            return jnp.dot(pltpu.bitcast(lhs, BF16),
                           pltpu.bitcast(jnp.concatenate(rhs, axis=0), BF16),
                           preferred_element_type=F32)

        def pack(lo, hi):
            return pltpu.bitcast(jnp.concatenate([lo, hi], axis=0).astype(BF16), U32)

        def halves(t):
            return [jnp.take_along_axis(t, spread + off, axis=1) for off in (0, 64)]

        def layernorm_lhs(x):
            m = jnp.sum(x, axis=1, keepdims=True) * (1.0 / d_model)
            xc = x - m
            v = jnp.sum(xc * xc, axis=1, keepdims=True) * (1.0 / d_model)
            rs = lax.rsqrt(v + EPS)
            out = []
            for t in range(ND):
                for g in halves(x[:, t * 128:(t + 1) * 128]):
                    n = (g - m) * rs
                    out.append(pack(jnp.where(lane_c == 0, n, 0.0),
                                    jnp.where(lane_c == 1, n, 0.0)))
            put("x", 0, out)

        def x_matmul(name, pairs, cp):
            acc = None
            for i in range(2 * ND):
                r = tile_matmul(load("x", 0, i),
                                [load(name, cp, (8 * i + a) * pairs) for a in range(8)])
                acc = r if acc is None else acc + r
                yield
            return acc[0:8], acc[8:16]

        def q_tiles(cp):
            out = []
            for t in (yield from x_matmul("wq", NQ // 2, cp)):
                for g in halves(t):
                    g = jnp.where(lane_c == (sub & 1), g, 0.0)
                    out.append(pack(g, g))
            return out

        def q_operand(h):
            return [load("q", h * (NA // 8), t) for t in range(NA // 8)]

        def scores(q, h, g):
            kh = h * HV
            s = None
            for j in range(4):
                r = None
                for t in range(NA // 8):
                    rhs = [load("k", kh, (8 * t + a) * NB + 4 * g + j) for a in range(8)]
                    d = tile_matmul(q[t], rhs)[0:8]
                    r = d if r is None else r + d
                    yield
                s = r if s is None else jnp.where((sub >> 1) == j, r, s)
            return s

        def all_scores(h):
            q = q_operand(h)
            return [_run(scores(q, h, g)) for g in range(NB // 4)]

        def softmax(parts):
            s = jnp.concatenate(parts, axis=0)
            m = jnp.max(jnp.max(s, axis=0, keepdims=True), axis=1, keepdims=True)
            e = jnp.exp((s - m) * (DH ** -0.5))
            den = jnp.sum(jnp.sum(e, axis=0, keepdims=True), axis=1, keepdims=True)
            return ([jnp.broadcast_to(e[i:i + 1, :], (8, 128)) for i in range(2 * NB)],
                    [jnp.broadcast_to(1.0 / den, (8, 128))])

        def put_softmax(parts, h, slot):
            e, r = softmax(parts)
            put("p", slot * (2 * NB), e)
            put("r", h, r)

        def p_times_v(h, slot, acc, after=None):
            vh = h * HV
            for a0 in range(0, NA, ACC):
                for b in range(NB):
                    p0, p1 = get("p", slot * (2 * NB), 2, 2 * b)
                    for i in range(ACC):
                        v = pltpu.bitcast(load("v", vh, (a0 + i) * NB + b), BF16).astype(F32)
                        t = v[0:8] * p0 + v[8:16] * p1
                        if b:
                            acc[i] = acc[i] + t
                        else:
                            acc[i] = t if acc[i] is None or not after else after(t, acc[i])
                    if b == NB - 1:
                        for i in range(ACC):
                            ab[slot, (a0 + i) * 8:(a0 + i + 1) * 8, :] = acc[i]
                    if (b + 1) * ACC % 8 == 0:
                        yield

        def retile(name, k0, n):
            def body(k, _):
                base = k * KT
                for g in range(8):
                    old = [load(name, base, g * ND + t) for t in range(ND)]
                    half = [v[4 * i:4 * i + 4] for v in old for i in range(2)]
                    for t in range(ND):
                        buf[base + (at[name] + g * ND + t)] = jnp.concatenate(
                            [half[t], half[ND + t]], axis=0)
            lax.fori_loop(k0, k0 + n, body, None)

        def row_matmul(lhs, name, base, k, y):
            out = []
            for t in range(ND):
                r = tile_matmul(lhs, [load(name, base, k * KT + g * ND + t)
                                      for g in range(8)])[0:8]
                out.append(r if y is None else y[t] + r)
                yield
            return out

        def head_outputs(pair):
            parts = jnp.concatenate([ab[0], ab[1]], axis=0)
            r0, r1 = get("r", 2 * pair, 2)
            out = []
            for j, r in enumerate((r0, jnp.where(lane < DH - 128, r0, r1), r1)):
                o = jnp.sum(parts[j * 128:(j + 1) * 128].T, axis=0, keepdims=True) * r
                out.append(pack(o, o))
            return out

        def out_proj(lhs, pair):
            base, y = pair * (3 * KT), None
            for j in range(3):
                y = yield from row_matmul(lhs[j], "wo", base, j, y)
            return y

        def add_out_proj(pair):
            y = _run(out_proj(head_outputs(pair), pair))
            return [a + b for a, b in zip(get("y", 0, ND), y)]

        def residual(x, y):
            y = jnp.concatenate(y, axis=1)
            return (x + y.astype(BF16).astype(F32)).astype(BF16).astype(F32)

        def glu_hidden(g, u):
            hid = jax.nn.sigmoid(g) * u
            return pack(hid, hid)

        def ff_matmul(name, cp):
            return _run(x_matmul(name, NF // 2, cp))

        zeros = [jnp.zeros((8, 128), F32)] * ND

        qn = sizes["wq"] // NSQ
        start("wq", 0, qn, S_Q)
        x_copy = pltpu.make_async_copy(x_hbm, xb, sems.at[S_X])
        x_copy.start()
        start("wq", qn, qn, S_Q + 1)
        x_copy.wait()
        x = jnp.broadcast_to(xb[...].astype(F32), (8, d_model))
        layernorm_lhs(x)
        put("y", 0, zeros)
        for s in range(NSQ):
            wait("wq", s * qn, qn, S_Q + s % 2)
            if s + 2 < NSQ:
                start("wq", (s + 2) * qn, qn, S_Q + s % 2)
            elif s + 2 == NSQ:
                start_head("k", 0, S_K)
            else:
                start_head("v", 0, S_V)

        def head1(h, _):
            odd = h & 1
            pair = h >> 1

            @pl.when(h < NQ // 2)
            def _():
                put("q", 4 * h, _run(q_tiles(h)))

            wait("k", h * HV, HV, S_K)

            @pl.when(h + 1 < HQ)
            def _():
                start_head("k", h + 1, S_K)

            @pl.when(h + 1 == HQ)
            def _():
                start("wg", 0, sizes["wg"], S_G)

            put_softmax(all_scores(h), h, odd)
            wait("v", h * HV, HV, S_V)

            @pl.when(h + 1 < HQ)
            def _():
                start_head("v", h + 1, S_V)

            @pl.when(h + 1 == HQ)
            def _():
                start("wu", 0, sizes["wu"], S_U)

            @pl.when(odd == 0)
            def _():
                start("wo", pair * (3 * KT), 3 * KT, S_O)

            _run(p_times_v(h, odd, [None] * ACC))

            @pl.when(odd == 1)
            def _():
                wait("wo", pair * (3 * KT), 3 * KT, S_O)
                retile("wo", 3 * pair, 3)
                put("y", 0, add_out_proj(pair))

        lax.fori_loop(0, HQ, head1, None)

        for i, (k0, k1) in enumerate(WD_PIECES):
            start("wd", k0 * KT, (k1 - k0) * KT, S_D + i)
        x = residual(x, get("y", 0, ND))
        layernorm_lhs(x)
        wait("wg", 0, sizes["wg"], S_G)
        gate = [t for cp in range(NF // 2) for t in ff_matmul("wg", cp)]
        wait("wu", 0, sizes["wu"], S_U)
        up = [t for cp in range(NF // 2) for t in ff_matmul("wu", cp)]
        hid = [glu_hidden(g, u) for g, u in zip(gate, up)]
        y = None
        for i, (k0, k1) in enumerate(WD_PIECES):
            wait("wd", k0 * KT, (k1 - k0) * KT, S_D + i)
            retile("wd", k0, k1 - k0)
            for k in range(k0, k1):
                y = _run(row_matmul(hid[k], "wd", 0, k, y))
        x = residual(x, y)

        layernorm_lhs(x)
        for cp in range(3):
            put("q", 4 * cp, _run(q_tiles(cp)))
        s0 = all_scores(0)
        put("s", 0, all_scores(1))
        put_softmax(s0, 0, 0)
        put("y", 0, zeros)

        def pair2(j, _):
            never = lane < (j >> 8)
            hc = jnp.minimum(2 * j + 2, HQ - 2)
            qc, qd = q_operand(hc), q_operand(hc + 1)
            put_softmax(get("s", 0, NB // 4), 2 * j + 1, 1)
            prev = head_outputs(jnp.maximum(j - 1, 0))
            now, due, second = [0], [], []

            def after(value, other):
                return jnp.where(never, pltpu.bitcast(other, F32), value)

            def ready(vals, extra=0):
                due.append((now[0] + DELAY + extra, vals))

            def mxu_stream():
                sc = []
                for g in range(NB // 4):
                    sc.append((yield from scores(qc, hc, g)))
                    ready(sc[-1:])
                pc, rc = softmax(sc)
                second.append(lambda: (put("p", 0, pc), put("r", 2 * j + 2, rc)))
                ready(pc[7::8], SM_DELAY)
                y = yield from out_proj(prev, jnp.maximum(j - 1, 0))
                y = [a + jnp.where(j > 0, b, 0.0) for a, b in zip(get("y", 0, ND), y)]
                put("y", 0, y)
                ready(y)
                for i in range(2):
                    cp = jnp.minimum(2 * j + 3 + i, NQ // 2 - 1)
                    q = yield from q_tiles(cp)
                    put("q", 4 * cp, q)
                    ready(q, 8)
                for g in range(NB // 4):
                    sd = yield from scores(qd, hc + 1, g)
                    put("s", g, [sd])
                    ready([sd])

            n_tiles = 2 * NB * NA // 8 + 3 * ND + 4 * ND
            mxu, issued, acc, turn = mxu_stream(), 0, [None] * ACC, 0
            for k in range(2):
                for _ in p_times_v(2 * j + k, k, acc, after if CHAIN else None):
                    now[0] += 1
                    while issued <= min(n_tiles, now[0] * n_tiles // MXU_SEGS):
                        next(mxu, None)
                        issued += 1
                    for item in [it for it in due if it[0] <= now[0]]:
                        due[:] = [it for it in due if it is not item]
                        for val in item[1]:
                            acc[turn % ACC] = after(acc[turn % ACC], val)
                            turn += 1
            second[0]()

        lax.fori_loop(0, HQ // 2, pair2, None)
        x = residual(x, add_out_proj(HQ // 2 - 1))

        layernorm_lhs(x)
        y = None
        for cp in range(NF // 2):
            gate, up = ff_matmul("wg", cp), ff_matmul("wu", cp)
            for c in range(2):
                y = _run(row_matmul(glu_hidden(gate[c], up[c]), "wd", 0, 2 * cp + c, y))
        o_ref[...] = residual(x, y)[0:1].astype(o_ref.dtype)

    scratch = [
        pltpu.VMEM((1, d_model), BF16),
        pltpu.VMEM((total, 8, 128), U32),
        pltpu.VMEM((2, DH, 128), F32),
        pltpu.SemaphoreType.DMA((n_sems,)),
    ] + [pltpu.VMEM((n, 8, 128), U32) for n in work.values()]
    return kernel, scratch


@jax.jit
def pallas_interleave_layers__sliding_block_cached__glu_gated_glu__decode_kernel(
    A_x: jax.Array,
    A_k_cache: jax.Array,
    A_v_cache: jax.Array,
    A_wq: jax.Array,
    A_wo: jax.Array,
    B_x: jax.Array,
    B_w_gate: jax.Array,
    B_w_up: jax.Array,
    B_w_down: jax.Array,
):
    del B_x
    d_model, d_ff = B_w_gate.shape
    sk = A_k_cache.shape[2]
    win = min(4096, max(256, sk // 4))
    assert A_x.shape == (1, 1, 640) and d_ff == 1536 and win == 4096
    assert A_k_cache.shape == A_v_cache.shape == (1, HQ, sk, DH) and sk % 256 == 0

    def cache_view(c):
        return _vreg_view(jnp.swapaxes(c, 2, 3).reshape(HQ, DH, sk))

    kernel, scratch = _make_kernel(d_model, d_ff, sk, win)
    out = pl.pallas_call(
        kernel,
        out_shape=jax.ShapeDtypeStruct((1, d_model), A_x.dtype),
        in_specs=[pl.BlockSpec(memory_space=pl.ANY)] * 8,
        out_specs=pl.BlockSpec(memory_space=pltpu.VMEM),
        scratch_shapes=scratch,
        compiler_params=pltpu.CompilerParams(vmem_limit_bytes=126 * 1024 * 1024),
        name="attn_glu_x2",
    )(A_x.reshape(1, d_model), cache_view(A_k_cache), cache_view(A_v_cache),
      *map(_vreg_view, (A_wq, A_wo, B_w_gate, B_w_up, B_w_down)))
    return out.reshape(A_x.shape)
```

```python
import functools

import jax
import jax.numpy as jnp
from jax import lax
import jax.experimental.pallas as pl
import jax.experimental.pallas.tpu as pltpu

F32 = jnp.float32
BF16 = jnp.bfloat16
U32 = jnp.uint32

HQ, DH = 32, 192
NA = DH // 8
CH = 8
EPS = 1e-5
SCALE = DH ** -0.5
LOWEST = -3e38
WD_PIECES = ((0, 6), (6, 10), (10, 11), (11, 12))
ACC = 8


def _vreg_view(w):
    *lead, r, c = w.shape
    n = len(lead)
    t = w.reshape(*lead, r // 8, 8, c // 128, 128)
    t = jnp.transpose(t, (*range(n), n, n + 2, n + 1, n + 3))
    return t.reshape(-1, 16, 128)


def _make_kernel(d_model, d_ff, sk, win):
    NB = win // 256
    HV = NA * NB
    ND = d_model // 128
    NF = d_ff // 128
    NQ = HQ * DH // 128
    KT = 8 * ND
    NSQ = 5
    S_K, S_V, S_O, S_Q = 0, 1, 2, 3
    S_G, S_U, S_X, S_D = S_K, S_V, S_O, S_Q
    n_sems = S_D + max(2, len(WD_PIECES))
    sizes = dict(k=HQ * HV, v=HQ * HV, wq=NQ * KT, wo=NQ * KT, wg=NF * KT, wu=NF * KT,
                 wd=NF * KT)
    work = dict(p0=2 * NB, p1=2 * NB, stat0=2, stat1=2, w0=1, w1=1, w=1, den0=1, den1=1, inv=2,
                pv=NA, o=3, y=ND, x=2 * ND, q=NQ, q_sum=4, spread=1,
                raw_s0=3 * NB, raw_s1=3 * NB, raw_q=8 * ND, raw_o=4, raw_y=3 * ND)
    at, n_vregs = {}, 0
    for name, size in sizes.items():
        at[name], n_vregs = n_vregs, n_vregs + size

    def kernel(x_hbm, k_hbm, v_hbm, wq_hbm, wo_hbm, wg_hbm, wu_hbm, wd_hbm, o_ref,
               xb, buf, sems, *work_refs):
        wk = dict(zip(work, work_refs))
        lane = lax.broadcasted_iota(jnp.int32, (8, 128), 1)
        sub = lax.broadcasted_iota(jnp.int32, (8, 128), 0)
        lane_c = (lane >> 3) & 1

        hbm = dict(k=k_hbm, v=v_hbm, wq=wq_hbm, wo=wo_hbm, wg=wg_hbm, wu=wu_hbm, wd=wd_hbm)
        hbm = {name: ref.bitcast(U32) for name, ref in hbm.items()}

        def piece(name, src, dst, sem, queue):
            pltpu.make_async_copy(hbm[name].at[pl.ds(src, CH)],
                                  buf.at[pl.ds(at[name] + dst, CH)],
                                  sems.at[sem]).start(priority=queue)

        def start(name, i0, n, sem):
            def body(j, _):
                for c in range(2):
                    piece(name, i0 + (2 * j + c) * CH, i0 + (2 * j + c) * CH, sem, c)
            lax.fori_loop(0, n // (2 * CH), body, None)
            if n // CH % 2:
                piece(name, i0 + n - CH, i0 + n - CH, sem, 0)

        def start_head(name, h, sem):
            def body(a, _):
                for c in range(NB // CH):
                    piece(name, (h * NA + a) * (sk // 256) + (sk // 256 - NB + c * CH),
                          (h * NA + a) * NB + c * CH, sem, c % 2)
            lax.fori_loop(0, NA, body, None, unroll=2)

        def wait(name, i0, n, sem):
            blk = buf.at[pl.ds(at[name] + i0, n)]
            pltpu.make_async_copy(blk, blk, sems.at[sem]).wait()

        def load(name, base, off):
            return buf[base + (at[name] + off)] if name in sizes else wk[name][base + off]

        def put(name, base, vals):
            for i, v in enumerate(vals):
                wk[name][base + i] = pltpu.bitcast(v, U32)

        def get(name, base, n, off=0):
            return [pltpu.bitcast(load(name, base, off + i), F32) for i in range(n)]

        def tile_matmul(lhs, rhs):
            return jnp.dot(pltpu.bitcast(lhs, BF16),
                           pltpu.bitcast(jnp.concatenate(rhs, axis=0), BF16),
                           preferred_element_type=F32)

        def pack(lo, hi):
            return pltpu.bitcast(jnp.concatenate([lo, hi], axis=0).astype(BF16), U32)

        def spread(t):
            idx = pltpu.bitcast(load("spread", 0, 0), jnp.int32)
            return jnp.take_along_axis(t, idx, axis=1, mode="promise_in_bounds",
                                       wrap_negative_indices=False)

        def layernorm_lhs(x):
            m = jnp.sum(x, axis=1, keepdims=True) * (1.0 / d_model)
            xc = x - m
            v = jnp.sum(xc * xc, axis=1, keepdims=True) * (1.0 / d_model)
            rs = lax.rsqrt(v + EPS)
            out = []
            for t in range(ND):
                both = (spread(x[:, t * 128:(t + 1) * 128]) - m) * rs
                for half in range(2):
                    n = jnp.broadcast_to(both[4 * half:4 * half + 1], (8, 128))
                    out.append(pack(jnp.where(lane_c == 0, n, 0.0),
                                    jnp.where(lane_c == 1, n, 0.0)))
            put("x", 0, out)

        def total(vals):
            return functools.reduce(jnp.add, vals)

        def x_tiles(name, pairs, cp):
            out = []
            for i in range(2 * ND):
                r = tile_matmul(load("x", 0, i),
                                [load(name, cp, (8 * i + a) * pairs) for a in range(8)])
                out += [r[0:8], r[8:16]]
            return out

        def x_matmul(name, pairs, cp):
            raw = x_tiles(name, pairs, cp)
            return total(raw[0::2]), total(raw[1::2])

        def put_q(cp, packed):
            keep = jnp.where(lane_c == 0, 0xFFFF, -0x10000)
            put("q", 2 * cp, [spread(pltpu.bitcast(t, jnp.int32)) & keep for t in packed])

        def make_q(cp):
            put_q(cp, [pack(t, t) for t in x_matmul("wq", NQ // 2, cp)])

        def score_tiles(hq, odd, base, dh):
            q = [load("q", (3 * hq) >> 1, i) for i in range(2)]
            out = []
            for b in range(NB):
                for t in range(NA // 8):
                    r = tile_matmul(q[(odd + t) // 2],
                                    [load("k", base, dh * HV + (8 * t + a) * NB + b)
                                     for a in range(8)])
                    out.append(r[8:16] if (odd + t) % 2 else r[0:8])
            return out

        def rows_of(v):
            return jnp.broadcast_to(v, (8, 128))

        def put_lane_softmax(raw, slot):
            parts = []
            for b in range(NB):
                r = total(raw[3 * b:3 * b + 3])
                if b % 4:
                    parts[-1] = jnp.where((sub >> 1) == b % 4, r, parts[-1])
                else:
                    parts.append(r)
            top = jnp.max(functools.reduce(jnp.maximum, parts), axis=0, keepdims=True)
            top = rows_of(jnp.maximum(top, LOWEST))
            e = [jnp.exp((s - top) * SCALE) for s in parts]
            put(f"p{slot}", 0, [rows_of(e[i // 8][i % 8:i % 8 + 1]) for i in range(2 * NB)])
            put(f"stat{slot}", 0, [top, rows_of(jnp.sum(total(e), axis=0, keepdims=True))])

        def put_lane_weights(slot):
            top, part = get(f"stat{slot}", 0, 2)
            w = jnp.exp((top - jnp.max(top, axis=1, keepdims=True)) * SCALE)
            w = w.astype(BF16).astype(F32)
            put(f"den{slot}", 0, [w * part])
            if slot:
                put("w", 0, [pack(get("w0", 0, 1)[0], w)])
            else:
                put("w0", 0, [w])

        def put_inverse(slot):
            den = jnp.sum(get(f"den{slot}", 0, 1)[0], axis=1, keepdims=True)
            put("inv", slot, [rows_of(1.0 / den)])

        def p_times_v(base, slot):
            for a0 in range(0, NA, ACC):
                acc = [None] * ACC
                for b in range(NB):
                    p0, p1 = get(f"p{slot}", 0, 2, 2 * b)
                    for i in range(ACC):
                        v = load("v", base, (a0 + i) * NB + b)
                        v = pltpu.bitcast(v, BF16).astype(F32)
                        t = v[0:8] * p0 + v[8:16] * p1
                        acc[i] = acc[i] + t if b else t
                put("pv", slot * (NA // 2) + a0 // 2,
                    [pack(acc[i], acc[i + 1]) for i in range(0, ACC, 2)])

        def retile(name, k0, n):
            def body(k, _):
                base = k * KT
                for g in range(8):
                    old = [load(name, base, g * ND + t) for t in range(ND)]
                    half = [v[4 * i:4 * i + 4] for v in old for i in range(2)]
                    for t in range(ND):
                        buf[base + (at[name] + g * ND + t)] = jnp.concatenate(
                            [half[t], half[ND + t]], axis=0)
            lax.fori_loop(k0, k0 + n, body, None)

        def row_tiles(lhs, name, base, k):
            return [tile_matmul(lhs, [load(name, base, k * KT + g * ND + t)
                                      for g in range(8)])[0:8] for t in range(ND)]

        def add_rows(y, raw):
            return [total(([] if y is None else [y[t]]) + raw[t::ND]) for t in range(ND)]

        def merge_lanes():
            w = pltpu.bitcast(load("w", 0, 0), BF16)
            out = []
            for j, keep in enumerate(((0,), (0, 8), (8,))):
                rhs = jnp.concatenate([load("pv", 0, 8 * j + i) for i in range(8)], axis=0)
                r = lax.dot_general(w, pltpu.bitcast(rhs, BF16), (((1,), (1,)), ((), ())),
                                    preferred_element_type=F32)
                out += [r[k:k + 8] for k in keep]
            return out

        def head_outputs(raw):
            r0, r1 = get("inv", 0, 2)
            out = (raw[0] * r0, jnp.where(lane < DH - 128, raw[1] * r0, raw[2] * r1),
                   raw[3] * r1)
            return [pack(o, o) for o in out]

        def out_tiles(lhs, pair):
            base = pair * (3 * KT)
            return [t for j in range(3) for t in row_tiles(lhs[j], "wo", base, j)]

        def residual(x, y):
            y = jnp.concatenate(y, axis=1)
            return (x + y.astype(BF16).astype(F32)).astype(BF16).astype(F32)

        def glu_hidden(g, u):
            hid = jax.nn.sigmoid(g) * u
            return pack(hid, hid)

        def ff_matmul(name, cp):
            return x_matmul(name, NF // 2, cp)

        zeros = [jnp.zeros((8, 128), F32)] * ND

        qn = sizes["wq"] // NSQ
        start("wq", 0, qn, S_Q)
        x_copy = pltpu.make_async_copy(x_hbm, xb, sems.at[S_X])
        x_copy.start()
        start("wq", qn, qn, S_Q + 1)
        put("spread", 0, [((sub >> 2) << 6) | ((lane >> 4) << 3) | (lane & 7)])
        x_copy.wait()
        x = jnp.broadcast_to(xb[...].astype(F32), (8, d_model))
        layernorm_lhs(x)
        put("y", 0, zeros)
        for s in range(NSQ):
            wait("wq", s * qn, qn, S_Q + s % 2)
            if s + 2 < NSQ:
                start("wq", (s + 2) * qn, qn, S_Q + s % 2)
            elif s + 2 == NSQ:
                start_head("k", 0, S_K)
            else:
                start_head("v", 0, S_V)

        def head1(h, _):
            odd = h & 1
            pair = h >> 1

            @pl.when(h < NQ // 2)
            def _():
                make_q(h)

            wait("k", h * HV, HV, S_K)

            @pl.when(h + 1 < HQ)
            def _():
                start_head("k", h + 1, S_K)

            @pl.when(h + 1 == HQ)
            def _():
                start("wg", 0, sizes["wg"], S_G)

            wait("v", h * HV, HV, S_V)

            @pl.when(h + 1 < HQ)
            def _():
                start_head("v", h + 1, S_V)

            @pl.when(h + 1 == HQ)
            def _():
                start("wu", 0, sizes["wu"], S_U)

            @pl.when(odd == 0)
            def _():
                start("wo", pair * (3 * KT), 3 * KT, S_O)

            for slot in range(2):
                @pl.when(odd == slot)
                def _():
                    put_lane_softmax(score_tiles(h, slot, h * HV, 0), slot)
                    put_lane_weights(slot)
                    put_inverse(slot)
                    p_times_v(h * HV, slot)

            @pl.when(odd == 1)
            def _():
                wait("wo", pair * (3 * KT), 3 * KT, S_O)
                retile("wo", 3 * pair, 3)
                lhs = head_outputs(merge_lanes())
                put("y", 0, add_rows(get("y", 0, ND), out_tiles(lhs, pair)))

        lax.fori_loop(0, HQ, head1, None)

        for i, (k0, k1) in enumerate(WD_PIECES):
            start("wd", k0 * KT, (k1 - k0) * KT, S_D + i)
        x = residual(x, get("y", 0, ND))
        layernorm_lhs(x)
        wait("wg", 0, sizes["wg"], S_G)
        gate = [t for cp in range(NF // 2) for t in ff_matmul("wg", cp)]
        wait("wu", 0, sizes["wu"], S_U)
        up = [t for cp in range(NF // 2) for t in ff_matmul("wu", cp)]
        hid = [glu_hidden(g, u) for g, u in zip(gate, up)]
        y = None
        for i, (k0, k1) in enumerate(WD_PIECES):
            wait("wd", k0 * KT, (k1 - k0) * KT, S_D + i)
            retile("wd", k0, k1 - k0)
            for k in range(k0, k1):
                y = add_rows(y, row_tiles(hid[k], "wd", 0, k))
        x = residual(x, y)

        layernorm_lhs(x)
        for cp in range(3):
            make_q(cp)
        put("raw_q", 0, [t for cp in (3, 4) for t in x_tiles("wq", NQ // 2, cp)])
        put_lane_softmax(score_tiles(0, 0, 0, 0), 0)
        put("raw_s1", 0, score_tiles(1, 1, 0, 1))
        put("y", 0, zeros)
        put("o", 0, zeros[:3])

        def head2(h, _):
            base, pair = h * HV, h >> 1

            def step(slot):
                put_lane_softmax(get(f"raw_s{1 - slot}", 0, 3 * NB), 1 - slot)
                put_lane_weights(slot)
                put_inverse(1 - slot)
                p_times_v(base, slot)
                put(f"raw_s{slot}", 0,
                    score_tiles(jnp.minimum(h + 2, HQ - 2 + slot), slot, base, 2))

            @pl.when(h & 1 == 0)
            def _():
                raw = get("raw_q", 0, 8 * ND)
                sums = [total(raw[i:i + 4 * ND:2]) for i in (0, 1, 4 * ND, 4 * ND + 1)]
                put("q_sum", 0, [pack(t, t) for t in sums])
                put("raw_o", 0, merge_lanes())
                step(0)
                put("raw_y", 0, out_tiles([load("o", 0, j) for j in range(3)],
                                          jnp.maximum(pair - 2, 0)))

            @pl.when(h & 1 == 1)
            def _():
                put("o", 0, head_outputs(get("raw_o", 0, 4)))
                new = add_rows(None, get("raw_y", 0, 3 * ND))
                put("y", 0, [a + jnp.where(pair > 1, b, 0.0)
                             for a, b in zip(get("y", 0, ND), new)])
                step(1)
                for i in range(2):
                    put_q(jnp.minimum(h + 2 + i, NQ // 2 - 1), get("q_sum", 0, 2, 2 * i))
                put("raw_q", 0, [t for i in range(2) for t in x_tiles(
                    "wq", NQ // 2, jnp.minimum(h + 4 + i, NQ // 2 - 1))])

        lax.fori_loop(0, HQ, head2, None)
        put_inverse(1)
        raw = merge_lanes()
        y = add_rows(get("y", 0, ND),
                     out_tiles([load("o", 0, j) for j in range(3)], HQ // 2 - 2))
        x = residual(x, add_rows(y, out_tiles(head_outputs(raw), HQ // 2 - 1)))

        layernorm_lhs(x)
        y = None
        for cp in range(NF // 2):
            gate, up = ff_matmul("wg", cp), ff_matmul("wu", cp)
            for c in range(2):
                hid = glu_hidden(gate[c], up[c])
                y = add_rows(y, row_tiles(hid, "wd", 0, 2 * cp + c))
        o_ref[...] = residual(x, y)[0:1].astype(o_ref.dtype)

    scratch = [
        pltpu.VMEM((1, d_model), BF16),
        pltpu.VMEM((n_vregs, 8, 128), U32),
        pltpu.SemaphoreType.DMA((n_sems,)),
    ] + [pltpu.VMEM((n, 8, 128), U32) for n in work.values()]
    return kernel, scratch


@jax.jit
def pallas_interleave_layers__sliding_block_cached__glu_gated_glu__decode_kernel(
    A_x: jax.Array,
    A_k_cache: jax.Array,
    A_v_cache: jax.Array,
    A_wq: jax.Array,
    A_wo: jax.Array,
    B_x: jax.Array,
    B_w_gate: jax.Array,
    B_w_up: jax.Array,
    B_w_down: jax.Array,
):
    del B_x
    d_model, d_ff = B_w_gate.shape
    sk = A_k_cache.shape[2]
    win = min(4096, max(256, sk // 4))
    assert A_x.shape == (1, 1, 640) and d_ff == 1536 and win == 4096
    assert A_k_cache.shape == A_v_cache.shape == (1, HQ, sk, DH) and sk % 256 == 0

    def cache_view(c):
        return _vreg_view(jnp.swapaxes(c, 2, 3).reshape(HQ, DH, sk))

    kernel, scratch = _make_kernel(d_model, d_ff, sk, win)
    out = pl.pallas_call(
        kernel,
        out_shape=jax.ShapeDtypeStruct((1, d_model), A_x.dtype),
        in_specs=[pl.BlockSpec(memory_space=pl.ANY)] * 8,
        out_specs=pl.BlockSpec(memory_space=pltpu.VMEM),
        scratch_shapes=scratch,
        compiler_params=pltpu.CompilerParams(vmem_limit_bytes=126 * 1024 * 1024),
        name="attn_glu_x2",
    )(A_x.reshape(1, d_model), cache_view(A_k_cache), cache_view(A_v_cache),
      *map(_vreg_view, (A_wq, A_wo, B_w_gate, B_w_up, B_w_down)))
    return out.reshape(A_x.shape)
```

```python
import functools
import itertools

import jax
import jax.numpy as jnp
from jax import lax
import jax.experimental.pallas as pl
import jax.experimental.pallas.tpu as pltpu

F32 = jnp.float32
BF16 = jnp.bfloat16
U32 = jnp.uint32

HQ, DH = 32, 192
NA = DH // 8
CH = 4
EPS = 1e-5
SCALE = DH ** -0.5
LOWEST = -3e38
WD_PIECES = ((0, 6), (6, 9), (9, 11), (11, 12))
ACC = 8
GLU_LAG = 2


def _vreg_view(w):
    *lead, r, c = w.shape
    n = len(lead)
    t = w.reshape(*lead, r // 8, 8, c // 128, 128)
    t = jnp.transpose(t, (*range(n), n, n + 2, n + 1, n + 3))
    return t.reshape(-1, 16, 128)


def _make_kernel(d_model, d_ff, sk, win):
    NB = win // 256
    HV = NA * NB
    ND = d_model // 128
    NF = d_ff // 128
    NQ = HQ * DH // 128
    KT = 8 * ND
    NSQ = 5
    S_K, S_V, S_O, S_Q = 0, 1, 2, 3
    S_G, S_U, S_X, S_D = S_K, S_V, S_O, S_Q
    n_sems = S_D + max(2, len(WD_PIECES))
    sizes = dict(k=HQ * HV, v=HQ * HV, wq=NQ * KT, wo=NQ * KT, wg=NF * KT, wu=NF * KT,
                 wd=NF * KT)
    work = dict(p0=2 * NB, p1=2 * NB, stat0=2, stat1=2, w0=1, w1=1, w=1, den0=1, den1=1, inv=2,
                pv=NA, o=3, y=ND, x=2 * ND, q=NQ, q_sum=4, spread=1,
                raw_s0=3 * NB, raw_s1=3 * NB, raw_q=8 * ND, raw_o=4, raw_y=3 * ND)
    at, n_vregs = {}, 0
    for name, size in sizes.items():
        at[name], n_vregs = n_vregs, n_vregs + size

    def kernel(x_hbm, k_hbm, v_hbm, wq_hbm, wo_hbm, wg_hbm, wu_hbm, wd_hbm, o_ref,
               xb, buf, sems, *work_refs):
        wk = dict(zip(work, work_refs))
        lane = lax.broadcasted_iota(jnp.int32, (8, 128), 1)
        sub = lax.broadcasted_iota(jnp.int32, (8, 128), 0)
        lane_c = (lane >> 3) & 1

        hbm = dict(k=k_hbm, v=v_hbm, wq=wq_hbm, wo=wo_hbm, wg=wg_hbm, wu=wu_hbm, wd=wd_hbm)
        hbm = {name: ref.bitcast(U32) for name, ref in hbm.items()}

        def streams(name, src, src_stride, dst, dst_stride, count, sem):
            def body(c, _):
                for i in range(count):
                    pltpu.make_async_copy(
                        hbm[name].at[pl.ds(src + c * CH + i * src_stride, CH)],
                        buf.at[pl.ds(dst + c * CH + (at[name] + i * dst_stride), CH)],
                        sems.at[sem]).start(priority=i % 2)
            lax.fori_loop(0, dst_stride // CH, body, None)

        def start(name, i0, n, sem):
            count = 6 if n % (6 * CH) == 0 else 2
            streams(name, i0, n // count, i0, n // count, count, sem)

        def start_head(name, h, sem):
            row = sk // 256
            streams(name, h * (NA * row) + (row - NB), row, h * HV, NB, NA, sem)

        def wait(name, i0, n, sem):
            blk = buf.at[pl.ds(at[name] + i0, n)]
            pltpu.make_async_copy(blk, blk, sems.at[sem]).wait()

        def load(name, base, off):
            return buf[base + (at[name] + off)] if name in sizes else wk[name][base + off]

        def put(name, base, vals):
            for i, v in enumerate(vals):
                wk[name][base + i] = pltpu.bitcast(v, U32)

        def get(name, base, n, off=0):
            return [pltpu.bitcast(load(name, base, off + i), F32) for i in range(n)]

        def tile_matmul(lhs, rhs):
            return jnp.dot(pltpu.bitcast(lhs, BF16),
                           pltpu.bitcast(jnp.concatenate(rhs, axis=0), BF16),
                           preferred_element_type=F32)

        def pack(lo, hi):
            return pltpu.bitcast(jnp.concatenate([lo, hi], axis=0).astype(BF16), U32)

        def spread(t):
            idx = pltpu.bitcast(load("spread", 0, 0), jnp.int32)
            return jnp.take_along_axis(t, idx, axis=1, mode="promise_in_bounds",
                                       wrap_negative_indices=False)

        def layernorm_lhs(x):
            m = jnp.sum(x, axis=1, keepdims=True) * (1.0 / d_model)
            xc = x - m
            v = jnp.sum(xc * xc, axis=1, keepdims=True) * (1.0 / d_model)
            rs = lax.rsqrt(v + EPS)
            out = []
            for t in range(ND):
                both = (spread(x[:, t * 128:(t + 1) * 128]) - m) * rs
                for half in range(2):
                    n = jnp.broadcast_to(both[4 * half:4 * half + 1], (8, 128))
                    out.append(pack(jnp.where(lane_c == 0, n, 0.0),
                                    jnp.where(lane_c == 1, n, 0.0)))
            put("x", 0, out)

        def total(vals):
            return functools.reduce(jnp.add, vals)

        def x_tiles(name, pairs, cp):
            out = []
            for i in range(2 * ND):
                r = tile_matmul(load("x", 0, i),
                                [load(name, cp, (8 * i + a) * pairs) for a in range(8)])
                out += [r[0:8], r[8:16]]
            return out

        def x_matmul(name, pairs, cp):
            raw = x_tiles(name, pairs, cp)
            return total(raw[0::2]), total(raw[1::2])

        def put_q(cp, packed):
            keep = jnp.where(lane_c == 0, 0xFFFF, -0x10000)
            put("q", 2 * cp, [spread(pltpu.bitcast(t, jnp.int32)) & keep for t in packed])

        def make_q(cp):
            put_q(cp, [pack(t, t) for t in x_matmul("wq", NQ // 2, cp)])

        def score_tiles(hq, odd, base, dh):
            q = [load("q", (3 * hq) >> 1, i) for i in range(2)]
            out = []
            for b in range(NB):
                for t in range(NA // 8):
                    r = tile_matmul(q[(odd + t) // 2],
                                    [load("k", base, dh * HV + (8 * t + a) * NB + b)
                                     for a in range(8)])
                    out.append(r[8:16] if (odd + t) % 2 else r[0:8])
            return out

        def rows_of(v):
            return jnp.broadcast_to(v, (8, 128))

        def lane_softmax(raw, slot):
            parts = []
            for b in range(NB):
                r = total(raw(b))
                if b % 4:
                    parts[-1] = jnp.where((sub >> 1) == b % 4, r, parts[-1])
                else:
                    parts.append(r)
                if b % 2:
                    yield
            top = jnp.max(functools.reduce(jnp.maximum, parts), axis=0, keepdims=True)
            top = rows_of(jnp.maximum(top, LOWEST))
            yield
            yield
            e = [jnp.exp((s - top) * SCALE) for s in parts]
            yield
            yield
            put(f"stat{slot}", 0, [top, rows_of(jnp.sum(total(e), axis=0, keepdims=True))])
            for i in range(2 * NB):
                put(f"p{slot}", i, [rows_of(e[i // 8][i % 8:i % 8 + 1])])
                if i % 4 == 3:
                    yield

        def put_lane_softmax(raw, slot):
            for _ in lane_softmax(lambda b: raw[3 * b:3 * b + 3], slot):
                pass

        def put_lane_weights(slot):
            top, part = get(f"stat{slot}", 0, 2)
            w = jnp.exp((top - jnp.max(top, axis=1, keepdims=True)) * SCALE)
            w = w.astype(BF16).astype(F32)
            put(f"den{slot}", 0, [w * part])
            if slot:
                put("w", 0, [pack(get("w0", 0, 1)[0], w)])
            else:
                put("w0", 0, [w])

        def put_inverse(slot):
            den = jnp.sum(get(f"den{slot}", 0, 1)[0], axis=1, keepdims=True)
            put("inv", slot, [rows_of(1.0 / den)])

        def p_times_v(base, slot, side=None):
            for a0 in range(0, NA, ACC):
                acc = [None] * ACC
                for b in range(NB):
                    p0, p1 = get(f"p{slot}", 0, 2, 2 * b)
                    for i in range(ACC):
                        v = load("v", base, (a0 + i) * NB + b)
                        v = pltpu.bitcast(v, BF16).astype(F32)
                        t = v[0:8] * p0 + v[8:16] * p1
                        acc[i] = acc[i] + t if b else t
                    if side is not None and (b + 1) * ACC % 8 == 0:
                        next(side, None)
                put("pv", slot * (NA // 2) + a0 // 2,
                    [pack(acc[i], acc[i + 1]) for i in range(0, ACC, 2)])

        def retile(name, k0, n):
            def body(k, _):
                base = k * KT
                for g in range(8):
                    old = [load(name, base, g * ND + t) for t in range(ND)]
                    half = [v[4 * i:4 * i + 4] for v in old for i in range(2)]
                    for t in range(ND):
                        buf[base + (at[name] + g * ND + t)] = jnp.concatenate(
                            [half[t], half[ND + t]], axis=0)
            lax.fori_loop(k0, k0 + n, body, None)

        def row_tiles(lhs, name, base, k):
            return [tile_matmul(lhs, [load(name, base, k * KT + g * ND + t)
                                      for g in range(8)])[0:8] for t in range(ND)]

        def add_rows(y, raw):
            return [total(([] if y is None else [y[t]]) + raw[t::ND]) for t in range(ND)]

        def merge_lanes():
            w = pltpu.bitcast(load("w", 0, 0), BF16)
            out = []
            for j, keep in enumerate(((0,), (0, 8), (8,))):
                rhs = jnp.concatenate([load("pv", 0, 8 * j + i) for i in range(8)], axis=0)
                r = lax.dot_general(w, pltpu.bitcast(rhs, BF16), (((1,), (1,)), ((), ())),
                                    preferred_element_type=F32)
                out += [r[k:k + 8] for k in keep]
            return out

        def head_outputs(raw):
            r0, r1 = get("inv", 0, 2)
            out = (raw[0] * r0, jnp.where(lane < DH - 128, raw[1] * r0, raw[2] * r1),
                   raw[3] * r1)
            return [pack(o, o) for o in out]

        def out_tiles(lhs, pair):
            base = pair * (3 * KT)
            return [t for j in range(3) for t in row_tiles(lhs[j], "wo", base, j)]

        def residual(x, y):
            y = jnp.concatenate(y, axis=1)
            return (x + y.astype(BF16).astype(F32)).astype(BF16).astype(F32)

        def glu_hidden(g, u):
            hid = jax.nn.sigmoid(g) * u
            return pack(hid, hid)

        def ff_matmul(name, cp):
            return x_matmul(name, NF // 2, cp)

        zeros = [jnp.zeros((8, 128), F32)] * ND

        qn = sizes["wq"] // NSQ
        start("wq", 0, qn, S_Q)
        x_copy = pltpu.make_async_copy(x_hbm, xb, sems.at[S_X])
        x_copy.start()
        start("wq", qn, qn, S_Q + 1)
        put("spread", 0, [((sub >> 2) << 6) | ((lane >> 4) << 3) | (lane & 7)])
        x_copy.wait()
        x = jnp.broadcast_to(xb[...].astype(F32), (8, d_model))
        layernorm_lhs(x)
        put("y", 0, zeros)
        for s in range(NSQ):
            wait("wq", s * qn, qn, S_Q + s % 2)
            if s + 2 < NSQ:
                start("wq", (s + 2) * qn, qn, S_Q + s % 2)
            elif s + 2 == NSQ:
                start_head("k", 0, S_K)
            else:
                start_head("v", 0, S_V)

        def head1(h, _):
            odd = h & 1
            pair = h >> 1

            @pl.when(h < NQ // 2)
            def _():
                make_q(h)

            wait("k", h * HV, HV, S_K)

            @pl.when(h + 1 < HQ)
            def _():
                start_head("k", h + 1, S_K)

            @pl.when(h + 1 == HQ)
            def _():
                start("wg", 0, sizes["wg"], S_G)

            for slot in range(2):
                @pl.when(odd == slot)
                def _():
                    put_lane_softmax(score_tiles(h, slot, h * HV, 0), slot)
                    put_lane_weights(slot)
                    put_inverse(slot)

            wait("v", h * HV, HV, S_V)

            @pl.when(h + 1 < HQ)
            def _():
                start_head("v", h + 1, S_V)

            @pl.when(h + 1 == HQ)
            def _():
                start("wu", 0, sizes["wu"], S_U)

            @pl.when(odd == 0)
            def _():
                start("wo", pair * (3 * KT), 3 * KT, S_O)
                p_times_v(h * HV, 0)

            @pl.when(odd == 1)
            def _():
                p_times_v(h * HV, 1)
                wait("wo", pair * (3 * KT), 3 * KT, S_O)
                retile("wo", 3 * pair, 3)
                lhs = head_outputs(merge_lanes())
                put("y", 0, add_rows(get("y", 0, ND), out_tiles(lhs, pair)))

        lax.fori_loop(0, HQ, head1, None)

        for i, (k0, k1) in enumerate(WD_PIECES):
            start("wd", k0 * KT, (k1 - k0) * KT, S_D + i)
        x = residual(x, get("y", 0, ND))
        layernorm_lhs(x)
        wait("wg", 0, sizes["wg"], S_G)
        gate = [t for cp in range(NF // 2) for t in ff_matmul("wg", cp)]
        wait("wu", 0, sizes["wu"], S_U)
        up = [t for cp in range(NF // 2) for t in ff_matmul("wu", cp)]
        hid = [glu_hidden(g, u) for g, u in zip(gate, up)]
        y = None
        for i, (k0, k1) in enumerate(WD_PIECES):
            wait("wd", k0 * KT, (k1 - k0) * KT, S_D + i)
            retile("wd", k0, k1 - k0)
            for k in range(k0, k1):
                y = add_rows(y, row_tiles(hid[k], "wd", 0, k))
        x = residual(x, y)

        layernorm_lhs(x)
        for cp in range(3):
            make_q(cp)
        put("raw_q", 0, [t for cp in (3, 4) for t in x_tiles("wq", NQ // 2, cp)])
        put_lane_softmax(score_tiles(0, 0, 0, 0), 0)
        put("raw_s1", 0, score_tiles(1, 1, 0, 1))
        put("y", 0, zeros)
        put("o", 0, zeros[:3])

        def pair2(pair, _):
            def step(slot, side):
                h = 2 * pair + slot
                base = h * HV
                put_lane_weights(slot)
                put_inverse(1 - slot)
                scores = lambda b: get(f"raw_s{1 - slot}", 0, 3, 3 * b)
                p_times_v(base, slot, itertools.chain(lane_softmax(scores, 1 - slot), side))
                put(f"raw_s{slot}", 0,
                    score_tiles(jnp.minimum(h + 2, HQ - 2 + slot), slot, base, 2))

            def even():
                def side():
                    for i, off in enumerate((0, 1, 4 * ND, 4 * ND + 1)):
                        t = total([get("raw_q", 0, 1, off + 2 * k)[0] for k in range(2 * ND)])
                        put("q_sum", i, [pack(t, t)])
                        yield

                put("raw_o", 0, merge_lanes())
                step(0, side())
                put("raw_y", 0, out_tiles([load("o", 0, j) for j in range(3)],
                                          jnp.maximum(pair - 2, 0)))

            def odd():
                h = 2 * pair + 1

                def side():
                    y = get("y", 0, ND)
                    for t in range(ND):
                        new = total([get("raw_y", 0, 1, j * ND + t)[0] for j in range(3)])
                        put("y", t, [y[t] + jnp.where(pair > 1, new, 0.0)])
                        yield

                put("o", 0, head_outputs(get("raw_o", 0, 4)))
                step(1, side())
                for i in range(2):
                    put_q(jnp.minimum(h + 2 + i, NQ // 2 - 1), get("q_sum", 0, 2, 2 * i))
                put("raw_q", 0, [t for i in range(2) for t in x_tiles(
                    "wq", NQ // 2, jnp.minimum(h + 4 + i, NQ // 2 - 1))])

            even()
            pl.when(pair >> 8 == 0)(odd)

        lax.fori_loop(0, HQ // 2, pair2, None)
        put_inverse(1)
        raw = merge_lanes()
        y = add_rows(get("y", 0, ND),
                     out_tiles([load("o", 0, j) for j in range(3)], HQ // 2 - 2))
        x = residual(x, add_rows(y, out_tiles(head_outputs(raw), HQ // 2 - 1)))

        layernorm_lhs(x)
        y, hid = None, []
        for cp in range(NF // 2 + GLU_LAG):
            if cp < NF // 2:
                hid += map(glu_hidden, ff_matmul("wg", cp), ff_matmul("wu", cp))
            for k in range(2 * (cp - GLU_LAG), 2 * (cp - GLU_LAG + 1)):
                if k >= 0:
                    y = add_rows(y, row_tiles(hid[k], "wd", 0, k))
        o_ref[...] = residual(x, y)[0:1].astype(o_ref.dtype)

    scratch = [
        pltpu.VMEM((1, d_model), BF16),
        pltpu.VMEM((n_vregs, 8, 128), U32),
        pltpu.SemaphoreType.DMA((n_sems,)),
    ] + [pltpu.VMEM((n, 8, 128), U32) for n in work.values()]
    return kernel, scratch


@jax.jit
def pallas_interleave_layers__sliding_block_cached__glu_gated_glu__decode_kernel(
    A_x: jax.Array,
    A_k_cache: jax.Array,
    A_v_cache: jax.Array,
    A_wq: jax.Array,
    A_wo: jax.Array,
    B_x: jax.Array,
    B_w_gate: jax.Array,
    B_w_up: jax.Array,
    B_w_down: jax.Array,
):
    del B_x
    d_model, d_ff = B_w_gate.shape
    sk = A_k_cache.shape[2]
    win = min(4096, max(256, sk // 4))
    assert A_x.shape == (1, 1, 640) and d_ff == 1536 and win == 4096
    assert A_k_cache.shape == A_v_cache.shape == (1, HQ, sk, DH) and sk % 256 == 0

    def cache_view(c):
        return _vreg_view(jnp.swapaxes(c, 2, 3).reshape(HQ, DH, sk))

    kernel, scratch = _make_kernel(d_model, d_ff, sk, win)
    out = pl.pallas_call(
        kernel,
        out_shape=jax.ShapeDtypeStruct((1, d_model), A_x.dtype),
        in_specs=[pl.BlockSpec(memory_space=pl.ANY)] * 8,
        out_specs=pl.BlockSpec(memory_space=pltpu.VMEM),
        scratch_shapes=scratch,
        compiler_params=pltpu.CompilerParams(vmem_limit_bytes=126 * 1024 * 1024,
                                             disable_bounds_checks=True),
        name="attn_glu_x2",
    )(A_x.reshape(1, d_model), cache_view(A_k_cache), cache_view(A_v_cache),
      *map(_vreg_view, (A_wq, A_wo, B_w_gate, B_w_up, B_w_down)))
    return out.reshape(A_x.shape)
```

```python
import functools
import itertools

import jax
import jax.numpy as jnp
from jax import lax
import jax.experimental.pallas as pl
import jax.experimental.pallas.tpu as pltpu

F32 = jnp.float32
BF16 = jnp.bfloat16
U32 = jnp.uint32

HQ, DH = 32, 192
NA = DH // 8
CH = 4
EPS = 1e-5
SCALE = DH ** -0.5
LOWEST = -3e38
WD_PIECES = ((0, 6), (6, 9), (9, 11), (11, 12))
ACC = 8
GLU_LAG = 2


def _vreg_view(w):
    *lead, r, c = w.shape
    n = len(lead)
    t = w.reshape(*lead, r // 8, 8, c // 128, 128)
    t = jnp.transpose(t, (*range(n), n, n + 2, n + 1, n + 3))
    return t.reshape(-1, 16, 128)


def _make_kernel(d_model, d_ff, sk, win):
    NB = win // 256
    HV = NA * NB
    ND = d_model // 128
    NF = d_ff // 128
    NQ = HQ * DH // 128
    KT = 8 * ND
    NSQ = 3
    qn = NQ // 2 // NSQ
    S_K, S_V, S_O, S_Q = 0, 1, 2, 3
    S_G, S_U, S_X, S_D = S_K, S_V, S_O, S_Q
    n_sems = S_D + max(2, len(WD_PIECES))
    sizes = dict(k=HQ * HV, v=HQ * HV, wo=NQ * KT, wg=NF * KT, wu=NF * KT,
                 wd=NF * KT)
    work = dict(p0=2 * NB, p1=2 * NB, stat0=2, stat1=2, w0=1, w1=1, w=1, den0=1, den1=1, inv=2,
                pv0=NA // 2, pv1=NA // 2, pv0_kept=NA // 2, o=3, y=ND, x=2 * ND, q=NQ, q_sum=4, spread=1,
                raw_s0=3 * NB, raw_s1=3 * NB, raw_q=8 * ND, raw_o=4, raw_y=3 * ND)
    at, n_vregs = {}, 0
    for name, size in sizes.items():
        at[name], n_vregs = n_vregs, n_vregs + size

    def kernel(x_hbm, k_hbm, v_hbm, wq_hbm, wo_hbm, wg_hbm, wu_hbm, wd_hbm, o_ref,
               xb, buf, wq, sems, *work_refs):
        wk = dict(zip(work, work_refs))
        lane = lax.broadcasted_iota(jnp.int32, (8, 128), 1)
        sub = lax.broadcasted_iota(jnp.int32, (8, 128), 0)
        lane_c = (lane >> 3) & 1

        hbm = dict(k=k_hbm, v=v_hbm, wq=wq_hbm, wo=wo_hbm, wg=wg_hbm, wu=wu_hbm, wd=wd_hbm)
        hbm = {name: ref.bitcast(U32) for name, ref in hbm.items()}

        def streams(name, src, src_stride, dst, dst_stride, count, sem):
            def body(c, _):
                for i in range(count):
                    pltpu.make_async_copy(
                        hbm[name].at[pl.ds(src + c * CH + i * src_stride, CH)],
                        buf.at[pl.ds(dst + c * CH + (at[name] + i * dst_stride), CH)],
                        sems.at[sem]).start(priority=i % 2)
            lax.fori_loop(0, dst_stride // CH, body, None)

        def start(name, i0, n, sem):
            count = 6 if n % (6 * CH) == 0 else 2
            streams(name, i0, n // count, i0, n // count, count, sem)

        def start_head(name, h, sem):
            row = sk // 256
            streams(name, h * (NA * row) + (row - NB), row, h * HV, NB, NA, sem)

        def start_wq(step, sem):
            part = 2 * KT // 4

            def body(j, _):
                for cp in range(step * qn, (step + 1) * qn, CH):
                    for i in range(4):
                        a = j + i * part
                        pltpu.make_async_copy(hbm["wq"].at[pl.ds(a * (NQ // 2) + cp, CH)],
                                              wq.at[pl.ds(cp, CH), a],
                                              sems.at[sem]).start(priority=i % 2)
            lax.fori_loop(0, part, body, None)

        def wait_wq(step, sem):
            blk = wq.at[pl.ds(step * qn, qn)]
            pltpu.make_async_copy(blk, blk, sems.at[sem]).wait()

        def wait(name, i0, n, sem):
            blk = buf.at[pl.ds(at[name] + i0, n)]
            pltpu.make_async_copy(blk, blk, sems.at[sem]).wait()

        def load(name, base, off):
            return buf[base + (at[name] + off)] if name in sizes else wk[name][base + off]

        def put(name, base, vals):
            for i, v in enumerate(vals):
                wk[name][base + i] = pltpu.bitcast(v, U32)

        def get(name, base, n, off=0):
            return [pltpu.bitcast(load(name, base, off + i), F32) for i in range(n)]

        def tile_matmul(lhs, rhs):
            return jnp.dot(pltpu.bitcast(lhs, BF16),
                           pltpu.bitcast(jnp.concatenate(rhs, axis=0), BF16),
                           preferred_element_type=F32)

        def pack(even, odd=None):
            odd = even if odd is None else odd
            return pltpu.bitcast(pltpu.pack_elementwise([even, odd], packed_dtype=BF16), U32)

        def spread(t):
            idx = pltpu.bitcast(load("spread", 0, 0), jnp.int32)
            return jnp.take_along_axis(t, idx, axis=1, mode="promise_in_bounds",
                                       wrap_negative_indices=False)

        def layernorm_lhs(x):
            m = jnp.sum(x, axis=1, keepdims=True) * (1.0 / d_model)
            xc = x - m
            v = jnp.sum(xc * xc, axis=1, keepdims=True) * (1.0 / d_model)
            rs = lax.rsqrt(v + EPS)
            out = []
            for t in range(ND):
                both = (spread(x[:, t * 128:(t + 1) * 128]) - m) * rs
                for half in range(2):
                    n = jnp.broadcast_to(both[4 * half:4 * half + 1], (8, 128))
                    out.append(pack(jnp.where(lane_c == (sub >> 2), n, 0.0)))
            put("x", 0, out)

        def total(vals):
            return functools.reduce(jnp.add, vals)

        def x_tiles(name, cp):
            out = []
            for i in range(2 * ND):
                rhs = [wq[cp, a] if name == "wq" else load(name, cp, a * (NF // 2))
                       for a in range(8 * i, 8 * i + 8)]
                r = tile_matmul(load("x", 0, i), rhs)
                out += [r[0:8], r[8:16]]
            return out

        def x_matmul(name, cp):
            raw = x_tiles(name, cp)
            return total(raw[0::2]), total(raw[1::2])

        def put_q(cp, packed):
            keep = jnp.where(lane_c == 0, 0xFFFF, -0x10000)
            put("q", 2 * cp, [spread(pltpu.bitcast(t, jnp.int32)) & keep for t in packed])

        def make_q(cp):
            put_q(cp, [pack(t) for t in x_matmul("wq", cp)])

        def score_tiles(hq, odd, base, dh):
            q = [load("q", (3 * hq) >> 1, i) for i in range(2)]
            out = []
            for b in range(NB):
                for t in range(NA // 8):
                    r = tile_matmul(q[(odd + t) // 2],
                                    [load("k", base, dh * HV + (8 * t + a) * NB + b)
                                     for a in range(8)])
                    out.append(r[8:16] if (odd + t) % 2 else r[0:8])
            return out

        def rows_of(v):
            return jnp.broadcast_to(v, (8, 128))

        def lane_softmax(raw, slot):
            parts = []
            for b in range(NB):
                r = total(raw(b))
                if b % 4:
                    parts[-1] = jnp.where((sub >> 1) == b % 4, r, parts[-1])
                else:
                    parts.append(r)
                if b % 2:
                    yield
            top = jnp.max(functools.reduce(jnp.maximum, parts), axis=0, keepdims=True)
            top = rows_of(jnp.maximum(top, LOWEST))
            yield
            yield
            e = [jnp.exp((s - top) * SCALE) for s in parts]
            yield
            yield
            put(f"stat{slot}", 0, [top, rows_of(jnp.sum(total(e), axis=0, keepdims=True))])
            for i in range(2 * NB):
                put(f"p{slot}", i, [rows_of(e[i // 8][i % 8:i % 8 + 1])])
                if i % 4 == 3:
                    yield

        def put_lane_softmax(raw, slot):
            for _ in lane_softmax(lambda b: raw[3 * b:3 * b + 3], slot):
                pass

        def put_lane_weights(slot):
            top, part = get(f"stat{slot}", 0, 2)
            w = jnp.exp((top - jnp.max(top, axis=1, keepdims=True)) * SCALE)
            w = w.astype(BF16).astype(F32)
            put(f"den{slot}", 0, [w * part])
            if slot:
                put("w", 0, [pack(jnp.where(sub < 4, get("w0", 0, 1)[0], w))])
            else:
                put("w0", 0, [w])

        def put_inverse(slot):
            den = jnp.sum(get(f"den{slot}", 0, 1)[0], axis=1, keepdims=True)
            put("inv", slot, [rows_of(1.0 / den)])

        def p_times_v(base, slot, side=None):
            for a0 in range(0, NA, ACC):
                acc = [None] * ACC
                for b in range(NB):
                    p0, p1 = get(f"p{slot}", 0, 2, 2 * b)
                    for i in range(ACC):
                        v = load("v", base, (a0 + i) * NB + b)
                        v = pltpu.bitcast(v, BF16).astype(F32)
                        t = v[0:8] * p0 + v[8:16] * p1
                        acc[i] = acc[i] + t if b else t
                    if side is not None and (b + 1) * ACC % 8 == 0:
                        next(side, None)
                put(f"pv{slot}", a0 // 2,
                    [pack(acc[i], acc[i + 1]) for i in range(0, ACC, 2)])

        def retile(name, k0, n, weave=False):
            def body(k, _):
                base = k * KT
                for g in range(8):
                    old = [load(name, base, g * ND + t) for t in range(ND)]
                    if weave:
                        old = [pltpu.bitcast(v, BF16).astype(F32) for v in old]
                    half = [part for v in old for part in jnp.split(v, 2)]
                    for t in range(ND):
                        two = half[t], half[ND + t]
                        buf[base + (at[name] + g * ND + t)] = (
                            pack(*two) if weave else jnp.concatenate(two, axis=0))
            lax.fori_loop(k0, k0 + n, body, None)

        def row_tiles(lhs, name, base, k):
            return [tile_matmul(lhs, [load(name, base, k * KT + g * ND + t)
                                      for g in range(8)])[0:8] for t in range(ND)]

        def add_rows(y, raw):
            return [total(([] if y is None else [y[t]]) + raw[t::ND]) for t in range(ND)]

        def merge_lanes(first):
            w = pltpu.bitcast(load("w", 0, 0), BF16)
            rows = [load(name, 0, i) for name in (first, "pv1") for i in range(NA // 2)]
            out = []
            for j, keep in enumerate(((0,), (0, 8), (8,))):
                rhs = jnp.concatenate(rows[8 * j:8 * j + 8], axis=0)
                r = lax.dot_general(w, pltpu.bitcast(rhs, BF16), (((1,), (1,)), ((), ())),
                                    preferred_element_type=F32)
                out += [r[k:k + 8] for k in keep]
            return out

        def head_outputs(raw):
            r0, r1 = get("inv", 0, 2)
            out = (raw[0] * r0, jnp.where(lane < DH - 128, raw[1] * r0, raw[2] * r1),
                   raw[3] * r1)
            return [pack(o) for o in out]

        def out_tiles(lhs, pair):
            base = pair * (3 * KT)
            return [t for j in range(3) for t in row_tiles(lhs[j], "wo", base, j)]

        def residual(x, y):
            y = jnp.concatenate(y, axis=1)
            return (x + y.astype(BF16).astype(F32)).astype(BF16).astype(F32)

        def glu_hidden(g, u):
            hid = jax.nn.sigmoid(g) * u
            return pack(hid)

        zeros = [jnp.zeros((8, 128), F32)] * ND

        start_wq(0, S_Q)
        x_copy = pltpu.make_async_copy(x_hbm, xb, sems.at[S_X])
        x_copy.start()
        start_wq(1, S_Q + 1)
        put("spread", 0, [((sub >> 2) << 6) | ((lane >> 4) << 3) | (lane & 7)])
        x_copy.wait()
        x = jnp.broadcast_to(xb[...].astype(F32), (8, d_model))
        layernorm_lhs(x)
        put("y", 0, zeros)
        for s in range(NSQ):
            wait_wq(s, S_Q + s % 2)
            if s + 2 < NSQ:
                start_wq(s + 2, S_Q + s % 2)
            elif s + 2 == NSQ:
                start_head("k", 0, S_K)
            else:
                start_head("v", 0, S_V)

        def head1(h, _):
            odd = h & 1
            pair = h >> 1

            @pl.when(h < NQ // 2)
            def _():
                make_q(h)

            wait("k", h * HV, HV, S_K)

            @pl.when(h + 1 < HQ)
            def _():
                start_head("k", h + 1, S_K)

            @pl.when(h + 1 == HQ)
            def _():
                start("wg", 0, sizes["wg"], S_G)

            for slot in range(2):
                @pl.when(odd == slot)
                def _():
                    put_lane_softmax(score_tiles(h, slot, h * HV, 0), slot)
                    put_lane_weights(slot)
                    put_inverse(slot)

            wait("v", h * HV, HV, S_V)

            @pl.when(h + 1 < HQ)
            def _():
                start_head("v", h + 1, S_V)

            @pl.when(h + 1 == HQ)
            def _():
                start("wu", 0, sizes["wu"], S_U)

            @pl.when(odd == 0)
            def _():
                start("wo", pair * (3 * KT), 3 * KT, S_O)
                p_times_v(h * HV, 0)

            @pl.when(odd == 1)
            def _():
                p_times_v(h * HV, 1)
                wait("wo", pair * (3 * KT), 3 * KT, S_O)
                retile("wo", 3 * pair, 3, weave=True)
                lhs = head_outputs(merge_lanes("pv0"))
                put("y", 0, add_rows(get("y", 0, ND), out_tiles(lhs, pair)))

        lax.fori_loop(0, HQ, head1, None)

        for i, (k0, k1) in enumerate(WD_PIECES):
            start("wd", k0 * KT, (k1 - k0) * KT, S_D + i)
        x = residual(x, get("y", 0, ND))
        layernorm_lhs(x)
        wait("wg", 0, sizes["wg"], S_G)
        gate = [t for cp in range(NF // 2) for t in x_matmul("wg", cp)]
        wait("wu", 0, sizes["wu"], S_U)
        up = [t for cp in range(NF // 2) for t in x_matmul("wu", cp)]
        hid = [glu_hidden(g, u) for g, u in zip(gate, up)]
        y = None
        for i, (k0, k1) in enumerate(WD_PIECES):
            wait("wd", k0 * KT, (k1 - k0) * KT, S_D + i)
            retile("wd", k0, k1 - k0)
            for k in range(k0, k1):
                y = add_rows(y, row_tiles(hid[k], "wd", 0, k))
        x = residual(x, y)

        layernorm_lhs(x)
        for cp in range(3):
            make_q(cp)
        put("raw_q", 0, [t for cp in (3, 4) for t in x_tiles("wq", cp)])
        put_lane_softmax(score_tiles(0, 0, 0, 0), 0)
        put("raw_s1", 0, score_tiles(1, 1, 0, 1))
        put("y", 0, zeros)
        put("o", 0, zeros[:3])
        put("pv0_kept", 0, zeros[:1] * (NA // 2))

        def pair2(pair, _):
            def step(slot, side):
                h = 2 * pair + slot
                base = h * HV
                put_lane_weights(slot)
                put_inverse(1 - slot)
                scores = lambda b: get(f"raw_s{1 - slot}", 0, 3, 3 * b)
                p_times_v(base, slot, itertools.chain(lane_softmax(scores, 1 - slot), side))
                put(f"raw_s{slot}", 0,
                    score_tiles(jnp.minimum(h + 2, HQ - 2 + slot), slot, base, 2))

            def even():
                def side():
                    for i, off in enumerate((0, 1, 4 * ND, 4 * ND + 1)):
                        t = total([get("raw_q", 0, 1, off + 2 * k)[0] for k in range(2 * ND)])
                        put("q_sum", i, [pack(t)])
                        yield

                put("raw_o", 0, merge_lanes("pv0_kept"))
                step(0, side())
                put("raw_y", 0, out_tiles([load("o", 0, j) for j in range(3)],
                                          jnp.maximum(pair - 2, 0)))

            def odd():
                h = 2 * pair + 1

                def side():
                    put("pv0_kept", 0, get("pv0", 0, NA // 2))
                    yield
                    y = get("y", 0, ND)
                    for t in range(ND):
                        new = total([get("raw_y", 0, 1, j * ND + t)[0] for j in range(3)])
                        put("y", t, [y[t] + jnp.where(pair > 1, new, 0.0)])
                        yield

                put("o", 0, head_outputs(get("raw_o", 0, 4)))
                step(1, side())
                for i in range(2):
                    put_q(jnp.minimum(h + 2 + i, NQ // 2 - 1), get("q_sum", 0, 2, 2 * i))
                put("raw_q", 0, [t for i in range(2) for t in x_tiles(
                    "wq", jnp.minimum(h + 4 + i, NQ // 2 - 1))])

            even()
            pl.when(pair >> 8 == 0)(odd)

        lax.fori_loop(0, HQ // 2, pair2, None)
        put_inverse(1)
        raw = merge_lanes("pv0")
        y = add_rows(get("y", 0, ND),
                     out_tiles([load("o", 0, j) for j in range(3)], HQ // 2 - 2))
        x = residual(x, add_rows(y, out_tiles(head_outputs(raw), HQ // 2 - 1)))

        layernorm_lhs(x)
        y, hid = None, []
        for cp in range(NF // 2 + GLU_LAG):
            if cp < NF // 2:
                hid += map(glu_hidden, x_matmul("wg", cp), x_matmul("wu", cp))
            for k in range(2 * (cp - GLU_LAG), 2 * (cp - GLU_LAG + 1)):
                if k >= 0:
                    y = add_rows(y, row_tiles(hid[k], "wd", 0, k))
        o_ref[...] = residual(x, y)[0:1].astype(o_ref.dtype)

    scratch = [
        pltpu.VMEM((1, d_model), BF16),
        pltpu.VMEM((n_vregs, 8, 128), U32),
        pltpu.VMEM((NQ // 2, 2 * KT, 8, 128), U32),
        pltpu.SemaphoreType.DMA((n_sems,)),
    ] + [pltpu.VMEM((n, 8, 128), U32) for n in work.values()]
    return kernel, scratch


@jax.jit
def pallas_interleave_layers__sliding_block_cached__glu_gated_glu__decode_kernel(
    A_x: jax.Array,
    A_k_cache: jax.Array,
    A_v_cache: jax.Array,
    A_wq: jax.Array,
    A_wo: jax.Array,
    B_x: jax.Array,
    B_w_gate: jax.Array,
    B_w_up: jax.Array,
    B_w_down: jax.Array,
):
    del B_x
    d_model, d_ff = B_w_gate.shape
    sk = A_k_cache.shape[2]
    win = min(4096, max(256, sk // 4))
    assert A_x.shape == (1, 1, 640) and d_ff == 1536 and win == 4096
    assert A_k_cache.shape == A_v_cache.shape == (1, HQ, sk, DH) and sk % 256 == 0

    def cache_view(c):
        return _vreg_view(jnp.swapaxes(c, 2, 3).reshape(HQ, DH, sk))

    kernel, scratch = _make_kernel(d_model, d_ff, sk, win)
    out = pl.pallas_call(
        kernel,
        out_shape=jax.ShapeDtypeStruct((1, d_model), A_x.dtype),
        in_specs=[pl.BlockSpec(memory_space=pl.ANY)] * 8,
        out_specs=pl.BlockSpec(memory_space=pltpu.VMEM),
        scratch_shapes=scratch,
        compiler_params=pltpu.CompilerParams(vmem_limit_bytes=126 * 1024 * 1024,
                                             disable_bounds_checks=True),
        name="attn_glu_x2",
    )(A_x.reshape(1, d_model), cache_view(A_k_cache), cache_view(A_v_cache),
      *map(_vreg_view, (A_wq, A_wo, B_w_gate, B_w_up, B_w_down)))
    return out.reshape(A_x.shape)
```

```python
import functools
import itertools

import jax
import jax.numpy as jnp
from jax import lax
import jax.experimental.pallas as pl
import jax.experimental.pallas.tpu as pltpu

F32 = jnp.float32
BF16 = jnp.bfloat16
U32 = jnp.uint32

HQ, DH = 32, 192
NA = DH // 8
CH = 4
EPS = 1e-5
SCALE = DH ** -0.5
LOWEST = -3e38
WD_PIECES = ((0, 6), (6, 9), (9, 11), (11, 12))
ACC = 8
GLU_LAG = 2


def _vreg_view(w):
    *lead, r, c = w.shape
    n = len(lead)
    t = w.reshape(*lead, r // 8, 8, c // 128, 128)
    t = jnp.transpose(t, (*range(n), n, n + 2, n + 1, n + 3))
    return t.reshape(-1, 16, 128)


def _make_kernel(d_model, d_ff, sk, win):
    NB = win // 256
    HV = NA * NB
    ND = d_model // 128
    NF = d_ff // 128
    NQ = HQ * DH // 128
    KT = 8 * ND
    NSQ = 3
    qn = NQ // 2 // NSQ
    S_K, S_V, S_O, S_Q = 0, 1, 2, 3
    S_G, S_U, S_X, S_D = S_K, S_V, S_O, S_Q
    n_sems = S_D + max(2, len(WD_PIECES))
    sizes = dict(k=HQ * HV, v=HQ * HV, wo=NQ * KT, wg=NF * KT, wu=NF * KT,
                 wd=NF * KT)
    work = dict(p0=2 * NB, p1=2 * NB, stat0=2, stat1=2, w0=1, w1=1, w=1, den0=1, den1=1, inv=2,
                pv0=NA // 2, pv1=NA // 2, pv0_kept=NA // 2, o=3, y=ND, x=2 * ND, rstd=1, q=NQ, q_sum=4, spread=1,
                raw_s0=3 * NB, raw_s1=3 * NB, raw_q=8 * ND, raw_o=4, raw_y=3 * ND)
    at, n_vregs = {}, 0
    for name, size in sizes.items():
        at[name], n_vregs = n_vregs, n_vregs + size

    def kernel(x_hbm, k_hbm, v_hbm, wq_hbm, wo_hbm, wg_hbm, wu_hbm, wd_hbm, o_ref,
               xb, buf, wq, sems, *work_refs):
        wk = dict(zip(work, work_refs))
        lane = lax.broadcasted_iota(jnp.int32, (8, 128), 1)
        sub = lax.broadcasted_iota(jnp.int32, (8, 128), 0)
        lane_c = (lane >> 3) & 1

        hbm = dict(k=k_hbm, v=v_hbm, wq=wq_hbm, wo=wo_hbm, wg=wg_hbm, wu=wu_hbm, wd=wd_hbm)
        hbm = {name: ref.bitcast(U32) for name, ref in hbm.items()}

        def streams(name, src, src_stride, dst, dst_stride, count, sem):
            def body(c, _):
                for i in range(count):
                    pltpu.make_async_copy(
                        hbm[name].at[pl.ds(src + c * CH + i * src_stride, CH)],
                        buf.at[pl.ds(dst + c * CH + (at[name] + i * dst_stride), CH)],
                        sems.at[sem]).start(priority=i % 2)
            lax.fori_loop(0, dst_stride // CH, body, None)

        def start(name, i0, n, sem):
            count = 6 if n % (6 * CH) == 0 else 2
            streams(name, i0, n // count, i0, n // count, count, sem)

        def start_head(name, h, sem):
            row = sk // 256
            streams(name, h * (NA * row) + (row - NB), row, h * HV, NB, NA, sem)

        def start_wq(step, sem):
            part = 2 * KT // 4

            def body(j, _):
                for cp in range(step * qn, (step + 1) * qn, CH):
                    for i in range(4):
                        a = j + i * part
                        pltpu.make_async_copy(hbm["wq"].at[pl.ds(a * (NQ // 2) + cp, CH)],
                                              wq.at[pl.ds(cp, CH), a],
                                              sems.at[sem]).start(priority=i % 2)
            lax.fori_loop(0, part, body, None)

        def wait_wq(step, sem):
            blk = wq.at[pl.ds(step * qn, qn)]
            pltpu.make_async_copy(blk, blk, sems.at[sem]).wait()

        def wait(name, i0, n, sem):
            blk = buf.at[pl.ds(at[name] + i0, n)]
            pltpu.make_async_copy(blk, blk, sems.at[sem]).wait()

        def load(name, base, off):
            return buf[base + (at[name] + off)] if name in sizes else wk[name][base + off]

        def put(name, base, vals):
            for i, v in enumerate(vals):
                wk[name][base + i] = pltpu.bitcast(v, U32)

        def get(name, base, n, off=0):
            return [pltpu.bitcast(load(name, base, off + i), F32) for i in range(n)]

        def tile_matmul(lhs, rhs):
            return jnp.dot(pltpu.bitcast(lhs, BF16),
                           pltpu.bitcast(jnp.concatenate(rhs, axis=0), BF16),
                           preferred_element_type=F32)

        def pack(even, odd=None):
            odd = even if odd is None else odd
            return pltpu.bitcast(pltpu.pack_elementwise([even, odd], packed_dtype=BF16), U32)

        def spread(t):
            idx = pltpu.bitcast(load("spread", 0, 0), jnp.int32)
            return jnp.take_along_axis(t, idx, axis=1, mode="promise_in_bounds",
                                       wrap_negative_indices=False)

        def layernorm_lhs(x):
            m = jnp.sum(x, axis=1, keepdims=True) * (1.0 / d_model)
            xc = x - m
            v = jnp.sum(xc * xc, axis=1, keepdims=True) * (1.0 / d_model)
            put("rstd", 0, [rows_of(lax.rsqrt(v + EPS))])
            out = []
            for t in range(ND):
                both = spread(x[:, t * 128:(t + 1) * 128]) - m
                for half in range(2):
                    n = rows_of(both[4 * half:4 * half + 1])
                    out.append(pack(jnp.where(lane_c == (sub >> 2), n, 0.0)))
            put("x", 0, out)

        def total(vals):
            return functools.reduce(jnp.add, vals)

        def x_tiles(name, cp):
            out = []
            for i in range(2 * ND):
                rhs = [wq[cp, a] if name == "wq" else load(name, cp, a * (NF // 2))
                       for a in range(8 * i, 8 * i + 8)]
                r = tile_matmul(load("x", 0, i), rhs)
                out += [r[0:8], r[8:16]]
            return out

        def x_matmul(name, cp):
            raw = x_tiles(name, cp)
            rstd, = get("rstd", 0, 1)
            return total(raw[0::2]) * rstd, total(raw[1::2]) * rstd

        def put_q(cp, packed):
            keep = jnp.where(lane_c == 0, 0xFFFF, -0x10000)
            put("q", 2 * cp, [spread(pltpu.bitcast(t, jnp.int32)) & keep for t in packed])

        def make_q(cp):
            put_q(cp, [pack(t) for t in x_matmul("wq", cp)])

        def score_tiles(hq, odd, base, dh):
            q = [load("q", (3 * hq) >> 1, i) for i in range(2)]
            out = []
            for b in range(NB):
                for t in range(NA // 8):
                    r = tile_matmul(q[(odd + t) // 2],
                                    [load("k", base, dh * HV + (8 * t + a) * NB + b)
                                     for a in range(8)])
                    out.append(r[8:16] if (odd + t) % 2 else r[0:8])
            return out

        def rows_of(v):
            return jnp.broadcast_to(v, (8, 128))

        def lane_softmax(raw, slot):
            parts = []
            for b in range(NB):
                r = total(raw(b))
                if b % 4:
                    parts[-1] = jnp.where((sub >> 1) == b % 4, r, parts[-1])
                else:
                    parts.append(r)
                if b % 2:
                    yield
            top = jnp.max(functools.reduce(jnp.maximum, parts), axis=0, keepdims=True)
            top = rows_of(jnp.maximum(top, LOWEST))
            yield
            yield
            e = [jnp.exp((s - top) * SCALE) for s in parts]
            yield
            yield
            put(f"stat{slot}", 0, [top, rows_of(jnp.sum(total(e), axis=0, keepdims=True))])
            for i in range(2 * NB):
                put(f"p{slot}", i, [rows_of(e[i // 8][i % 8:i % 8 + 1])])
                if i % 4 == 3:
                    yield

        def put_lane_softmax(raw, slot):
            for _ in lane_softmax(lambda b: raw[3 * b:3 * b + 3], slot):
                pass

        def put_lane_weights(slot):
            top, part = get(f"stat{slot}", 0, 2)
            w = jnp.exp((top - jnp.max(top, axis=1, keepdims=True)) * SCALE)
            w = w.astype(BF16).astype(F32)
            put(f"den{slot}", 0, [w * part])
            if slot:
                put("w", 0, [pack(jnp.where(sub < 4, get("w0", 0, 1)[0], w))])
            else:
                put("w0", 0, [w])

        def put_inverse(slot):
            den = jnp.sum(get(f"den{slot}", 0, 1)[0], axis=1, keepdims=True)
            put("inv", slot, [rows_of(1.0 / den)])

        def p_times_v(base, slot, side=None):
            for a0 in range(0, NA, ACC):
                acc = [None] * ACC
                for b in range(NB):
                    p0, p1 = get(f"p{slot}", 0, 2, 2 * b)
                    for i in range(ACC):
                        v = load("v", base, (a0 + i) * NB + b)
                        v = pltpu.bitcast(v, BF16).astype(F32)
                        t = v[0:8] * p0
                        acc[i] = (acc[i] + t if b else t) + v[8:16] * p1
                    if side is not None and (b + 1) * ACC % 8 == 0:
                        next(side, None)
                put(f"pv{slot}", a0 // 2,
                    [pack(acc[i], acc[i + 1]) for i in range(0, ACC, 2)])

        def retile(name, k0, n, weave=False):
            def body(k, _):
                base = k * KT
                for g in range(8):
                    old = [load(name, base, g * ND + t) for t in range(ND)]
                    if weave:
                        old = [pltpu.bitcast(v, BF16).astype(F32) for v in old]
                    half = [part for v in old for part in jnp.split(v, 2)]
                    for t in range(ND):
                        two = half[t], half[ND + t]
                        buf[base + (at[name] + g * ND + t)] = (
                            pack(*two) if weave else jnp.concatenate(two, axis=0))
            if n == 1:
                body(k0, None)
            else:
                lax.fori_loop(k0, k0 + n, body, None)

        def row_tiles(lhs, name, base, k):
            return [tile_matmul(lhs, [load(name, base, k * KT + g * ND + t)
                                      for g in range(8)])[0:8] for t in range(ND)]

        def add_rows(y, raw):
            return [total(([] if y is None else [y[t]]) + raw[t::ND]) for t in range(ND)]

        def merge_lanes(first):
            w = pltpu.bitcast(load("w", 0, 0), BF16)
            rows = [load(name, 0, i) for name in (first, "pv1") for i in range(NA // 2)]
            out = []
            for j, keep in enumerate(((0,), (0, 8), (8,))):
                rhs = jnp.concatenate(rows[8 * j:8 * j + 8], axis=0)
                r = lax.dot_general(w, pltpu.bitcast(rhs, BF16), (((1,), (1,)), ((), ())),
                                    preferred_element_type=F32)
                out += [r[k:k + 8] for k in keep]
            return out

        def head_outputs(raw):
            r0, r1 = get("inv", 0, 2)
            out = (raw[0] * r0, jnp.where(lane < DH - 128, raw[1] * r0, raw[2] * r1),
                   raw[3] * r1)
            return [pack(o) for o in out]

        def out_tiles(lhs, pair):
            base = pair * (3 * KT)
            return [t for j in range(3) for t in row_tiles(lhs[j], "wo", base, j)]

        def residual(x, y):
            y = jnp.concatenate(y, axis=1)
            return (x + y.astype(BF16).astype(F32)).astype(BF16).astype(F32)

        def glu_hidden(g, u):
            hid = jax.nn.sigmoid(g) * u
            return pack(hid)

        zeros = [jnp.zeros((8, 128), F32)] * ND

        start_wq(0, S_Q)
        x_copy = pltpu.make_async_copy(x_hbm, xb, sems.at[S_X])
        x_copy.start()
        start_wq(1, S_Q + 1)
        put("spread", 0, [((sub >> 2) << 6) | ((lane >> 4) << 3) | (lane & 7)])
        x_copy.wait()
        x = jnp.broadcast_to(xb[...].astype(F32), (8, d_model))
        layernorm_lhs(x)
        put("y", 0, zeros)
        for s in range(NSQ):
            wait_wq(s, S_Q + s % 2)
            if s + 2 < NSQ:
                start_wq(s + 2, S_Q + s % 2)
            elif s + 2 == NSQ:
                start_head("k", 0, S_K)
            else:
                start_head("v", 0, S_V)

        def head1(h, _):
            odd = h & 1
            pair = h >> 1

            @pl.when(h < NQ // 2)
            def _():
                make_q(h)

            wait("k", h * HV, HV, S_K)

            @pl.when(h + 1 < HQ)
            def _():
                start_head("k", h + 1, S_K)

            @pl.when(h + 1 == HQ)
            def _():
                start("wg", 0, sizes["wg"], S_G)

            for slot in range(2):
                @pl.when(odd == slot)
                def _():
                    put_lane_softmax(score_tiles(h, slot, h * HV, 0), slot)
                    put_lane_weights(slot)
                    put_inverse(slot)

            wait("v", h * HV, HV, S_V)

            @pl.when(h + 1 < HQ)
            def _():
                start_head("v", h + 1, S_V)

            @pl.when(h + 1 == HQ)
            def _():
                start("wu", 0, sizes["wu"], S_U)

            @pl.when(odd == 0)
            def _():
                start("wo", pair * (3 * KT), 3 * KT, S_O)
                p_times_v(h * HV, 0)

            @pl.when(odd == 1)
            def _():
                p_times_v(h * HV, 1)
                wait("wo", pair * (3 * KT), 3 * KT, S_O)
                retile("wo", 3 * pair, 3, weave=True)
                lhs = head_outputs(merge_lanes("pv0"))
                put("y", 0, add_rows(get("y", 0, ND), out_tiles(lhs, pair)))

        lax.fori_loop(0, HQ, head1, None)

        for i, (k0, k1) in enumerate(WD_PIECES):
            start("wd", k0 * KT, (k1 - k0) * KT, S_D + i)
        x = residual(x, get("y", 0, ND))
        layernorm_lhs(x)
        wait("wg", 0, sizes["wg"], S_G)
        gate = [t for cp in range(NF // 2) for t in x_matmul("wg", cp)]
        wait("wu", 0, sizes["wu"], S_U)
        up = [t for cp in range(NF // 2) for t in x_matmul("wu", cp)]
        hid = [glu_hidden(g, u) for g, u in zip(gate, up)]
        y = None
        for i, (k0, k1) in enumerate(WD_PIECES):
            wait("wd", k0 * KT, (k1 - k0) * KT, S_D + i)
            retile("wd", k0, k1 - k0)
            for k in range(k0, k1):
                y = add_rows(y, row_tiles(hid[k], "wd", 0, k))
        x = residual(x, y)

        layernorm_lhs(x)
        for cp in range(3):
            make_q(cp)
        put("raw_q", 0, [t for cp in (3, 4) for t in x_tiles("wq", cp)])
        put_lane_softmax(score_tiles(0, 0, 0, 0), 0)
        put("raw_s1", 0, score_tiles(1, 1, 0, 1))
        put("y", 0, zeros)
        put("o", 0, zeros[:3])
        put("pv0_kept", 0, zeros[:1] * (NA // 2))

        def pair2(more_q, pair, _):
            def step(slot, side):
                h = 2 * pair + slot
                base = h * HV
                put_lane_weights(slot)
                put_inverse(1 - slot)
                scores = lambda b: get(f"raw_s{1 - slot}", 0, 3, 3 * b)
                p_times_v(base, slot, itertools.chain(lane_softmax(scores, 1 - slot), side))
                put(f"raw_s{slot}", 0,
                    score_tiles(jnp.minimum(h + 2, HQ - 2 + slot), slot, base, 2))

            def even():
                def side():
                    for i, off in enumerate((0, 1, 4 * ND, 4 * ND + 1)):
                        t = total([get("raw_q", 0, 1, off + 2 * k)[0] for k in range(2 * ND)])
                        put("q_sum", i, [pack(t * get("rstd", 0, 1)[0])])
                        yield

                put("raw_o", 0, merge_lanes("pv0_kept"))
                step(0, side())
                put("raw_y", 0, out_tiles([load("o", 0, j) for j in range(3)],
                                          jnp.maximum(pair - 2, 0)))

            def odd():
                h = 2 * pair + 1

                def side():
                    put("pv0_kept", 0, get("pv0", 0, NA // 2))
                    yield
                    y = get("y", 0, ND)
                    for t in range(ND):
                        new = total([get("raw_y", 0, 1, j * ND + t)[0] for j in range(3)])
                        put("y", t, [y[t] + jnp.where(pair > 1, new, 0.0)])
                        yield

                put("o", 0, head_outputs(get("raw_o", 0, 4)))
                step(1, side())
                for i in range(2):
                    put_q(jnp.minimum(h + 2 + i, NQ // 2 - 1), get("q_sum", 0, 2, 2 * i))
                if more_q:
                    put("raw_q", 0, [t for i in range(2) for t in x_tiles(
                        "wq", jnp.minimum(h + 4 + i, NQ // 2 - 1))])

            even()
            pl.when(pair >> 8 == 0)(odd)

        q_done = (NQ // 2 - 4) // 2
        lax.fori_loop(0, q_done, functools.partial(pair2, True), None)
        lax.fori_loop(q_done, HQ // 2, functools.partial(pair2, False), None)
        put_inverse(1)
        raw = merge_lanes("pv0")
        y = add_rows(get("y", 0, ND),
                     out_tiles([load("o", 0, j) for j in range(3)], HQ // 2 - 2))
        x = residual(x, add_rows(y, out_tiles(head_outputs(raw), HQ // 2 - 1)))

        layernorm_lhs(x)
        y, hid = None, []
        for cp in range(NF // 2 + GLU_LAG):
            if cp < NF // 2:
                hid += map(glu_hidden, x_matmul("wg", cp), x_matmul("wu", cp))
            for k in range(2 * (cp - GLU_LAG), 2 * (cp - GLU_LAG + 1)):
                if k >= 0:
                    y = add_rows(y, row_tiles(hid[k], "wd", 0, k))
        o_ref[...] = residual(x, y)[0:1].astype(o_ref.dtype)

    scratch = [
        pltpu.VMEM((1, d_model), BF16),
        pltpu.VMEM((n_vregs, 8, 128), U32),
        pltpu.VMEM((NQ // 2, 2 * KT, 8, 128), U32),
        pltpu.SemaphoreType.DMA((n_sems,)),
    ] + [pltpu.VMEM((n, 8, 128), U32) for n in work.values()]
    return kernel, scratch


@jax.jit
def pallas_interleave_layers__sliding_block_cached__glu_gated_glu__decode_kernel(
    A_x: jax.Array,
    A_k_cache: jax.Array,
    A_v_cache: jax.Array,
    A_wq: jax.Array,
    A_wo: jax.Array,
    B_x: jax.Array,
    B_w_gate: jax.Array,
    B_w_up: jax.Array,
    B_w_down: jax.Array,
):
    del B_x
    d_model, d_ff = B_w_gate.shape
    sk = A_k_cache.shape[2]
    win = min(4096, max(256, sk // 4))
    assert A_x.shape == (1, 1, 640) and d_ff == 1536 and win == 4096
    assert A_k_cache.shape == A_v_cache.shape == (1, HQ, sk, DH) and sk % 256 == 0

    def cache_view(c):
        return _vreg_view(jnp.swapaxes(c, 2, 3).reshape(HQ, DH, sk))

    kernel, scratch = _make_kernel(d_model, d_ff, sk, win)
    out = pl.pallas_call(
        kernel,
        out_shape=jax.ShapeDtypeStruct((1, d_model), A_x.dtype),
        in_specs=[pl.BlockSpec(memory_space=pl.ANY)] * 8,
        out_specs=pl.BlockSpec(memory_space=pltpu.VMEM),
        scratch_shapes=scratch,
        compiler_params=pltpu.CompilerParams(vmem_limit_bytes=126 * 1024 * 1024,
                                             disable_bounds_checks=True),
        name="attn_glu_x2",
    )(A_x.reshape(1, d_model), cache_view(A_k_cache), cache_view(A_v_cache),
      *map(_vreg_view, (A_wq, A_wo, B_w_gate, B_w_up, B_w_down)))
    return out.reshape(A_x.shape)
```

```python
import functools
import itertools

import jax
import jax.numpy as jnp
from jax import lax
import jax.experimental.pallas as pl
import jax.experimental.pallas.tpu as pltpu

F32 = jnp.float32
BF16 = jnp.bfloat16
U32 = jnp.uint32

HQ, DH = 32, 192
NA = DH // 8
CH = 4
EPS = 1e-5
SCALE = DH ** -0.5
LOWEST = -3e38
WD_PIECES = ((0, 6), (6, 9), (9, 11), (11, 12))
ACC = 8
GLU_LAG = 2


def _vreg_view(w):
    *lead, r, c = w.shape
    n = len(lead)
    t = w.reshape(*lead, r // 8, 8, c // 128, 128)
    t = jnp.transpose(t, (*range(n), n, n + 2, n + 1, n + 3))
    return t.reshape(-1, 16, 128)


def _make_kernel(d_model, d_ff, sk, win):
    NB = win // 256
    HV = NA * NB
    ND = d_model // 128
    NF = d_ff // 128
    NQ = HQ * DH // 128
    KT = 8 * ND
    NSQ = 3
    qn = NQ // 2 // NSQ
    S_K, S_V, S_O, S_Q = 0, 1, 2, 3
    S_G, S_U, S_X, S_D = S_K, S_V, S_O, S_Q
    n_sems = S_D + max(2, len(WD_PIECES))
    sizes = dict(k=HQ * HV, v=HQ * HV, wo=NQ * KT, wg=NF * KT, wu=NF * KT,
                 wd=NF * KT)
    work = dict(p0=2 * NB, p1=2 * NB, stat0=2, stat1=2, w0=1, w1=1, w=1, den0=1, den1=1, inv=2,
                pv0=NA // 2, pv1=NA // 2, pv0_kept=NA // 2, o=3, y=ND, x=2 * ND, rstd=1, q=NQ, q_sum=4, spread=1,
                raw_s0=3 * NB, raw_s1=3 * NB, raw_q=8 * ND, raw_o=4, raw_y=3 * ND)
    at, n_vregs = {}, 0
    for name, size in sizes.items():
        at[name], n_vregs = n_vregs, n_vregs + size

    def kernel(x_hbm, k_hbm, v_hbm, wq_hbm, wo_hbm, wg_hbm, wu_hbm, wd_hbm, o_ref,
               xb, buf, wq, sems, *work_refs):
        wk = dict(zip(work, work_refs))
        lane = lax.broadcasted_iota(jnp.int32, (8, 128), 1)
        sub = lax.broadcasted_iota(jnp.int32, (8, 128), 0)
        lane_c = (lane >> 3) & 1

        hbm = dict(k=k_hbm, v=v_hbm, wq=wq_hbm, wo=wo_hbm, wg=wg_hbm, wu=wu_hbm, wd=wd_hbm)
        hbm = {name: ref.bitcast(U32) for name, ref in hbm.items()}

        def streams(name, src, src_stride, dst, dst_stride, count, sem):
            def body(c, _):
                for i in range(count):
                    pltpu.make_async_copy(
                        hbm[name].at[pl.ds(src + c * CH + i * src_stride, CH)],
                        buf.at[pl.ds(dst + c * CH + (at[name] + i * dst_stride), CH)],
                        sems.at[sem]).start(priority=i % 2)
            lax.fori_loop(0, dst_stride // CH, body, None)

        def start(name, i0, n, sem):
            count = 6 if n % (6 * CH) == 0 else 2
            streams(name, i0, n // count, i0, n // count, count, sem)

        def start_head(name, h, sem):
            row = sk // 256
            streams(name, h * (NA * row) + (row - NB), row, h * HV, NB, NA, sem)

        def start_wq(step, sem):
            part = 2 * KT // 4

            def body(j, _):
                for cp in range(step * qn, (step + 1) * qn, CH):
                    for i in range(4):
                        a = j + i * part
                        pltpu.make_async_copy(hbm["wq"].at[pl.ds(a * (NQ // 2) + cp, CH)],
                                              wq.at[pl.ds(cp, CH), a],
                                              sems.at[sem]).start(priority=i % 2)
            lax.fori_loop(0, part, body, None)

        def wait_wq(step, sem):
            blk = wq.at[pl.ds(step * qn, qn)]
            pltpu.make_async_copy(blk, blk, sems.at[sem]).wait()

        def wait(name, i0, n, sem):
            blk = buf.at[pl.ds(at[name] + i0, n)]
            pltpu.make_async_copy(blk, blk, sems.at[sem]).wait()

        def load(name, base, off):
            return buf[base + (at[name] + off)] if name in sizes else wk[name][base + off]

        def put(name, base, vals):
            for i, v in enumerate(vals):
                wk[name][base + i] = pltpu.bitcast(v, U32)

        def get(name, base, n, off=0):
            return [pltpu.bitcast(load(name, base, off + i), F32) for i in range(n)]

        def tile_matmul(lhs, rhs, contract=0):
            if lhs.dtype != F32:
                lhs = pltpu.bitcast(lhs, BF16)
            return lax.dot_general(lhs, pltpu.bitcast(jnp.concatenate(rhs, axis=0), BF16),
                                   (((1,), (contract,)), ((), ())), preferred_element_type=F32)

        def pack(even, odd=None):
            odd = even if odd is None else odd
            return pltpu.bitcast(pltpu.pack_elementwise([even, odd], packed_dtype=BF16), U32)

        def spread(t):
            idx = pltpu.bitcast(load("spread", 0, 0), jnp.int32)
            return jnp.take_along_axis(t, idx, axis=1, mode="promise_in_bounds",
                                       wrap_negative_indices=False)

        def layernorm_lhs(x):
            m = jnp.sum(x, axis=1, keepdims=True) * (1.0 / d_model)
            xc = x - m
            v = jnp.sum(xc * xc, axis=1, keepdims=True) * (1.0 / d_model)
            put("rstd", 0, [rows_of(lax.rsqrt(v + EPS))])
            out = []
            for t in range(ND):
                both = spread(x[:, t * 128:(t + 1) * 128]) - m
                for half in range(2):
                    n = rows_of(both[4 * half:4 * half + 1])
                    out.append(pack(jnp.where(lane_c == (sub >> 2), n, 0.0)))
            put("x", 0, out)

        def total(vals):
            return functools.reduce(jnp.add, vals)

        def x_tiles(name, cp):
            out = []
            for i in range(2 * ND):
                rhs = [wq[cp, a] if name == "wq" else load(name, cp, a * (NF // 2))
                       for a in range(8 * i, 8 * i + 8)]
                r = tile_matmul(load("x", 0, i), rhs)
                out += [r[0:8], r[8:16]]
            return out

        def x_matmul(name, cp):
            raw = x_tiles(name, cp)
            rstd, = get("rstd", 0, 1)
            return total(raw[0::2]) * rstd, total(raw[1::2]) * rstd

        def put_q(cp, packed):
            keep = jnp.where(lane_c == 0, 0xFFFF, -0x10000)
            put("q", 2 * cp, [spread(pltpu.bitcast(t, jnp.int32)) & keep for t in packed])

        def make_q(cp):
            put_q(cp, [pack(t) for t in x_matmul("wq", cp)])

        def score_tiles(hq, odd, base, dh):
            q = [load("q", (3 * hq) >> 1, i) for i in range(2)]
            out = []
            for b in range(NB):
                for t in range(NA // 8):
                    r = tile_matmul(q[(odd + t) // 2],
                                    [load("k", base, dh * HV + (8 * t + a) * NB + b)
                                     for a in range(8)])
                    out.append(r[8:16] if (odd + t) % 2 else r[0:8])
            return out

        def rows_of(v):
            return jnp.broadcast_to(v, (8, 128))

        def lane_softmax(raw, slot):
            parts = []
            for b in range(NB):
                r = total(raw(b))
                if b % 4:
                    parts[-1] = jnp.where((sub >> 1) == b % 4, r, parts[-1])
                else:
                    parts.append(r)
                if b % 2:
                    yield
            top = jnp.max(functools.reduce(jnp.maximum, parts), axis=0, keepdims=True)
            top = rows_of(jnp.maximum(top, LOWEST))
            yield
            yield
            e = [jnp.exp((s - top) * SCALE) for s in parts]
            yield
            yield
            put(f"stat{slot}", 0, [top, rows_of(jnp.sum(total(e), axis=0, keepdims=True))])
            for i in range(2 * NB):
                put(f"p{slot}", i, [rows_of(e[i // 8][i % 8:i % 8 + 1])])
                if i % 4 == 3:
                    yield

        def put_lane_softmax(raw, slot):
            for _ in lane_softmax(lambda b: raw[3 * b:3 * b + 3], slot):
                pass

        def put_lane_weights(slot):
            top, part = get(f"stat{slot}", 0, 2)
            w = jnp.exp((top - jnp.max(top, axis=1, keepdims=True)) * SCALE)
            w = w.astype(BF16).astype(F32)
            put(f"den{slot}", 0, [w * part])
            if slot:
                put("w", 0, [pack(jnp.where(sub < 4, get("w0", 0, 1)[0], w))])
            else:
                put("w0", 0, [w])

        def put_inverse(slot):
            den = jnp.sum(get(f"den{slot}", 0, 1)[0], axis=1, keepdims=True)
            put("inv", slot, [rows_of(1.0 / den)])

        def p_times_v(base, slot, side=None):
            for a0 in range(0, NA, ACC):
                acc = [None] * ACC
                for b in range(NB):
                    p0, p1 = get(f"p{slot}", 0, 2, 2 * b)
                    for i in range(ACC):
                        v = load("v", base, (a0 + i) * NB + b)
                        v = pltpu.bitcast(v, BF16).astype(F32)
                        t = v[0:8] * p0
                        acc[i] = (acc[i] + t if b else t) + v[8:16] * p1
                    if side is not None and (b + 1) * ACC % 8 == 0:
                        next(side, None)
                put(f"pv{slot}", a0 // 2,
                    [pack(acc[i], acc[i + 1]) for i in range(0, ACC, 2)])

        def retile(name, k0, n, weave=False):
            def body(k, _):
                base = k * KT
                for g in range(8):
                    old = [load(name, base, g * ND + t) for t in range(ND)]
                    if weave:
                        old = [pltpu.bitcast(v, BF16).astype(F32) for v in old]
                    half = [part for v in old for part in jnp.split(v, 2)]
                    for t in range(ND):
                        two = half[t], half[ND + t]
                        buf[base + (at[name] + g * ND + t)] = (
                            pack(*two) if weave else jnp.concatenate(two, axis=0))
            if n == 1:
                body(k0, None)
            else:
                lax.fori_loop(k0, k0 + n, body, None)

        def row_tiles(lhs, name, base, k):
            return [tile_matmul(lhs, [load(name, base, k * KT + g * ND + t)
                                      for g in range(8)]) for t in range(ND)]

        def add_rows(y, raw):
            return [total(([] if y is None else [y[t]]) + raw[t::ND]) for t in range(ND)]

        def merge_lanes(first):
            w = load("w", 0, 0)
            rows = [load(name, 0, i) for name in (first, "pv1") for i in range(NA // 2)]
            out = []
            for j, keep in enumerate(((0,), (0, 8), (8,))):
                r = tile_matmul(w, rows[8 * j:8 * j + 8], contract=1)
                out += [r[k:k + 8] for k in keep]
            return out

        def head_outputs(raw):
            r0, r1 = get("inv", 0, 2)
            return [raw[0] * r0, jnp.where(lane < DH - 128, raw[1] * r0, raw[2] * r1),
                    raw[3] * r1]

        def out_tiles(lhs, pair):
            base = pair * (3 * KT)
            return [t for j in range(3) for t in row_tiles(lhs[j], "wo", base, j)]

        def residual(x, y):
            y = jnp.concatenate(y, axis=1)
            return (x + y.astype(BF16).astype(F32)).astype(BF16).astype(F32)

        def glu_hidden(g, u):
            return jax.nn.sigmoid(g) * u

        zeros = [jnp.zeros((8, 128), F32)] * ND

        start_wq(0, S_Q)
        x_copy = pltpu.make_async_copy(x_hbm, xb, sems.at[S_X])
        x_copy.start()
        start_wq(1, S_Q + 1)
        put("spread", 0, [((sub >> 2) << 6) | ((lane >> 4) << 3) | (lane & 7)])
        x_copy.wait()
        x = jnp.broadcast_to(xb[...].astype(F32), (8, d_model))
        layernorm_lhs(x)
        put("y", 0, zeros)
        for s in range(NSQ):
            wait_wq(s, S_Q + s % 2)
            if s + 2 < NSQ:
                start_wq(s + 2, S_Q + s % 2)
            elif s + 2 == NSQ:
                start_head("k", 0, S_K)
            else:
                start_head("v", 0, S_V)

        def head1(h, _):
            odd = h & 1
            pair = h >> 1

            @pl.when(h < NQ // 2)
            def _():
                make_q(h)

            wait("k", h * HV, HV, S_K)

            @pl.when(h + 1 < HQ)
            def _():
                start_head("k", h + 1, S_K)

            @pl.when(h + 1 == HQ)
            def _():
                start("wg", 0, sizes["wg"], S_G)

            for slot in range(2):
                @pl.when(odd == slot)
                def _():
                    put_lane_softmax(score_tiles(h, slot, h * HV, 0), slot)
                    put_lane_weights(slot)
                    put_inverse(slot)

            wait("v", h * HV, HV, S_V)

            @pl.when(h + 1 < HQ)
            def _():
                start_head("v", h + 1, S_V)

            @pl.when(h + 1 == HQ)
            def _():
                start("wu", 0, sizes["wu"], S_U)

            @pl.when(odd == 0)
            def _():
                start("wo", pair * (3 * KT), 3 * KT, S_O)
                p_times_v(h * HV, 0)

            @pl.when(odd == 1)
            def _():
                p_times_v(h * HV, 1)
                wait("wo", pair * (3 * KT), 3 * KT, S_O)
                retile("wo", 3 * pair, 3, weave=True)
                lhs = head_outputs(merge_lanes("pv0"))
                put("y", 0, add_rows(get("y", 0, ND), out_tiles(lhs, pair)))

        lax.fori_loop(0, HQ, head1, None)

        for i, (k0, k1) in enumerate(WD_PIECES):
            start("wd", k0 * KT, (k1 - k0) * KT, S_D + i)
        x = residual(x, get("y", 0, ND))
        layernorm_lhs(x)
        wait("wg", 0, sizes["wg"], S_G)
        gate = [t for cp in range(NF // 2) for t in x_matmul("wg", cp)]
        wait("wu", 0, sizes["wu"], S_U)
        up = [t for cp in range(NF // 2) for t in x_matmul("wu", cp)]
        hid = [glu_hidden(g, u) for g, u in zip(gate, up)]
        y = None
        for i, (k0, k1) in enumerate(WD_PIECES):
            wait("wd", k0 * KT, (k1 - k0) * KT, S_D + i)
            retile("wd", k0, k1 - k0)
            for k in range(k0, k1):
                y = add_rows(y, row_tiles(hid[k], "wd", 0, k))
        x = residual(x, y)

        layernorm_lhs(x)
        for cp in range(3):
            make_q(cp)
        put("raw_q", 0, [t for cp in (3, 4) for t in x_tiles("wq", cp)])
        put_lane_softmax(score_tiles(0, 0, 0, 0), 0)
        put("raw_s1", 0, score_tiles(1, 1, 0, 1))
        put("y", 0, zeros)
        put("o", 0, zeros[:3])
        put("pv0_kept", 0, zeros[:1] * (NA // 2))

        def pair2(more_q, pair, _):
            def step(slot, side):
                h = 2 * pair + slot
                base = h * HV
                put_lane_weights(slot)
                put_inverse(1 - slot)
                scores = lambda b: get(f"raw_s{1 - slot}", 0, 3, 3 * b)
                p_times_v(base, slot, itertools.chain(lane_softmax(scores, 1 - slot), side))
                put(f"raw_s{slot}", 0,
                    score_tiles(jnp.minimum(h + 2, HQ - 2 + slot), slot, base, 2))

            def even():
                def side():
                    for i, off in enumerate((0, 1, 4 * ND, 4 * ND + 1)):
                        t = total([get("raw_q", 0, 1, off + 2 * k)[0] for k in range(2 * ND)])
                        put("q_sum", i, [pack(t * get("rstd", 0, 1)[0])])
                        yield

                put("raw_o", 0, merge_lanes("pv0_kept"))
                step(0, side())
                put("raw_y", 0, out_tiles(get("o", 0, 3),
                                          jnp.maximum(pair - 2, 0)))

            def odd():
                h = 2 * pair + 1

                def side():
                    put("pv0_kept", 0, get("pv0", 0, NA // 2))
                    yield
                    y = get("y", 0, ND)
                    for t in range(ND):
                        new = total([get("raw_y", 0, 1, j * ND + t)[0] for j in range(3)])
                        put("y", t, [y[t] + jnp.where(pair > 1, new, 0.0)])
                        yield

                put("o", 0, head_outputs(get("raw_o", 0, 4)))
                step(1, side())
                for i in range(2):
                    put_q(jnp.minimum(h + 2 + i, NQ // 2 - 1), get("q_sum", 0, 2, 2 * i))
                if more_q:
                    put("raw_q", 0, [t for i in range(2) for t in x_tiles(
                        "wq", jnp.minimum(h + 4 + i, NQ // 2 - 1))])

            even()
            pl.when(pair >> 8 == 0)(odd)

        q_done = (NQ // 2 - 4) // 2
        lax.fori_loop(0, q_done, functools.partial(pair2, True), None)
        lax.fori_loop(q_done, HQ // 2, functools.partial(pair2, False), None)
        put_inverse(1)
        raw = merge_lanes("pv0")
        y = add_rows(get("y", 0, ND),
                     out_tiles(get("o", 0, 3), HQ // 2 - 2))
        x = residual(x, add_rows(y, out_tiles(head_outputs(raw), HQ // 2 - 1)))

        layernorm_lhs(x)
        y, hid = None, []
        for cp in range(NF // 2 + GLU_LAG):
            if cp < NF // 2:
                hid += map(glu_hidden, x_matmul("wg", cp), x_matmul("wu", cp))
            for k in range(2 * (cp - GLU_LAG), 2 * (cp - GLU_LAG + 1)):
                if k >= 0:
                    y = add_rows(y, row_tiles(hid[k], "wd", 0, k))
        o_ref[...] = residual(x, y)[0:1].astype(o_ref.dtype)

    scratch = [
        pltpu.VMEM((1, d_model), BF16),
        pltpu.VMEM((n_vregs, 8, 128), U32),
        pltpu.VMEM((NQ // 2, 2 * KT, 8, 128), U32),
        pltpu.SemaphoreType.DMA((n_sems,)),
    ] + [pltpu.VMEM((n, 8, 128), U32) for n in work.values()]
    return kernel, scratch


@jax.jit
def pallas_interleave_layers__sliding_block_cached__glu_gated_glu__decode_kernel(
    A_x: jax.Array,
    A_k_cache: jax.Array,
    A_v_cache: jax.Array,
    A_wq: jax.Array,
    A_wo: jax.Array,
    B_x: jax.Array,
    B_w_gate: jax.Array,
    B_w_up: jax.Array,
    B_w_down: jax.Array,
):
    del B_x
    d_model, d_ff = B_w_gate.shape
    sk = A_k_cache.shape[2]
    win = min(4096, max(256, sk // 4))
    assert A_x.shape == (1, 1, 640) and d_ff == 1536 and win == 4096
    assert A_k_cache.shape == A_v_cache.shape == (1, HQ, sk, DH) and sk % 256 == 0

    def cache_view(c):
        return _vreg_view(jnp.swapaxes(c, 2, 3).reshape(HQ, DH, sk))

    kernel, scratch = _make_kernel(d_model, d_ff, sk, win)
    out = pl.pallas_call(
        kernel,
        out_shape=jax.ShapeDtypeStruct((1, d_model), A_x.dtype),
        in_specs=[pl.BlockSpec(memory_space=pl.ANY)] * 8,
        out_specs=pl.BlockSpec(memory_space=pltpu.VMEM),
        scratch_shapes=scratch,
        compiler_params=pltpu.CompilerParams(vmem_limit_bytes=126 * 1024 * 1024,
                                             disable_bounds_checks=True),
        name="attn_glu_x2",
    )(A_x.reshape(1, d_model), cache_view(A_k_cache), cache_view(A_v_cache),
      *map(_vreg_view, (A_wq, A_wo, B_w_gate, B_w_up, B_w_down)))
    return out.reshape(A_x.shape)
```

```python
import functools
import itertools

import jax
import jax.numpy as jnp
from jax import lax
import jax.experimental.pallas as pl
import jax.experimental.pallas.tpu as pltpu

F32 = jnp.float32
BF16 = jnp.bfloat16
U32 = jnp.uint32

HQ, DH = 32, 192
NA = DH // 8
CH = 4
EPS = 1e-5
SCALE = DH ** -0.5
LOWEST = -3e38
WD_PIECES = ((0, 6), (6, 9), (9, 11), (11, 12))
ACC = 8
GLU_LAG = 2


def _vreg_view(w):
    *lead, r, c = w.shape
    n = len(lead)
    t = w.reshape(*lead, r // 8, 8, c // 128, 128)
    t = jnp.transpose(t, (*range(n), n, n + 2, n + 1, n + 3))
    return t.reshape(-1, 16, 128)


def _make_kernel(d_model, d_ff, sk, win):
    NB = win // 256
    HV = NA * NB
    ND = d_model // 128
    NF = d_ff // 128
    NQ = HQ * DH // 128
    KT = 8 * ND
    NSQ = 3
    qn = NQ // 2 // NSQ
    S_K, S_V, S_O, S_Q = 0, 1, 2, 3
    S_G, S_U, S_X, S_D = S_K, S_V, S_O, S_Q
    n_sems = S_D + max(2, len(WD_PIECES))
    sizes = dict(k=HQ * HV, v=HQ * HV, wo=NQ * KT, wg=NF * KT, wu=NF * KT,
                 wd=NF * KT)
    work = dict(p0=2 * NB, p1=2 * NB, stat0=2, stat1=2, w=2, den0=1, den1=1, inv=2,
                o=3, y=ND, x=2 * ND, rstd=1, q=NQ, q_sum=4, spread=1,
                raw_s0=3 * NB, raw_s1=3 * NB, raw_q=8 * ND, raw_o=4, raw_y=3 * ND)
    at, n_vregs = {}, 0
    for name, size in sizes.items():
        at[name], n_vregs = n_vregs, n_vregs + size

    def kernel(x_hbm, k_hbm, v_hbm, wq_hbm, wo_hbm, wg_hbm, wu_hbm, wd_hbm, o_ref,
               xb, buf, wq, pv, pv_new, sems, *work_refs):
        wk = dict(zip(work, work_refs))
        lane = lax.broadcasted_iota(jnp.int32, (8, 128), 1)
        sub = lax.broadcasted_iota(jnp.int32, (8, 128), 0)
        lane_c = (lane >> 3) & 1

        hbm = dict(k=k_hbm, v=v_hbm, wq=wq_hbm, wo=wo_hbm, wg=wg_hbm, wu=wu_hbm, wd=wd_hbm)
        hbm = {name: ref.bitcast(U32) for name, ref in hbm.items()}

        def streams(name, src, src_stride, dst, dst_stride, count, sem):
            def body(c, _):
                for i in range(count):
                    pltpu.make_async_copy(
                        hbm[name].at[pl.ds(src + c * CH + i * src_stride, CH)],
                        buf.at[pl.ds(dst + c * CH + (at[name] + i * dst_stride), CH)],
                        sems.at[sem]).start(priority=i % 2)
            lax.fori_loop(0, dst_stride // CH, body, None)

        def start(name, i0, n, sem):
            count = 6 if n % (6 * CH) == 0 else 2
            streams(name, i0, n // count, i0, n // count, count, sem)

        def start_head(name, h, sem):
            row = sk // 256
            streams(name, h * (NA * row) + (row - NB), row, h * HV, NB, NA, sem)

        def start_wq(step, sem):
            part = 2 * KT // 4

            def body(j, _):
                for cp in range(step * qn, (step + 1) * qn, CH):
                    for i in range(4):
                        a = j + i * part
                        pltpu.make_async_copy(hbm["wq"].at[pl.ds(a * (NQ // 2) + cp, CH)],
                                              wq.at[pl.ds(cp, CH), a],
                                              sems.at[sem]).start(priority=i % 2)
            lax.fori_loop(0, part, body, None)

        def wait_wq(step, sem):
            blk = wq.at[pl.ds(step * qn, qn)]
            pltpu.make_async_copy(blk, blk, sems.at[sem]).wait()

        def wait(name, i0, n, sem):
            blk = buf.at[pl.ds(at[name] + i0, n)]
            pltpu.make_async_copy(blk, blk, sems.at[sem]).wait()

        def load(name, base, off):
            return buf[base + (at[name] + off)] if name in sizes else wk[name][base + off]

        def put(name, base, vals):
            for i, v in enumerate(vals):
                wk[name][base + i] = pltpu.bitcast(v, U32)

        def get(name, base, n, off=0):
            return [pltpu.bitcast(load(name, base, off + i), F32) for i in range(n)]

        def tile_matmul(lhs, rhs):
            if lhs.dtype != F32:
                lhs = pltpu.bitcast(lhs, BF16)
            return lax.dot_general(lhs, pltpu.bitcast(jnp.concatenate(rhs, axis=0), BF16),
                                   (((1,), (0,)), ((), ())), preferred_element_type=F32)

        def pack(top, bottom=None):
            bottom = top if bottom is None else bottom
            return pltpu.bitcast(jnp.concatenate([top, bottom], axis=0).astype(BF16), U32)

        def spread(t):
            idx = pltpu.bitcast(load("spread", 0, 0), jnp.int32)
            return jnp.take_along_axis(t, idx, axis=1, mode="promise_in_bounds",
                                       wrap_negative_indices=False)

        def layernorm_lhs(x):
            m = jnp.sum(x, axis=1, keepdims=True) * (1.0 / d_model)
            xc = x - m
            v = jnp.sum(xc * xc, axis=1, keepdims=True) * (1.0 / d_model)
            put("rstd", 0, [rows_of(lax.rsqrt(v + EPS))])
            out = []
            for t in range(ND):
                both = spread(x[:, t * 128:(t + 1) * 128]) - m
                for half in range(2):
                    n = rows_of(both[4 * half:4 * half + 1])
                    out.append(pack(*(jnp.where(lane_c == c, n, 0.0) for c in range(2))))
            put("x", 0, out)

        def total(vals):
            return functools.reduce(jnp.add, vals)

        def x_tiles(name, cp):
            out = []
            for i in range(2 * ND):
                rhs = [wq[cp, a] if name == "wq" else load(name, cp, a * (NF // 2))
                       for a in range(8 * i, 8 * i + 8)]
                r = tile_matmul(load("x", 0, i), rhs)
                out += [r[0:8], r[8:16]]
            return out

        def x_matmul(name, cp):
            raw = x_tiles(name, cp)
            rstd, = get("rstd", 0, 1)
            return total(raw[0::2]) * rstd, total(raw[1::2]) * rstd

        def put_q(cp, packed):
            keep = jnp.where(lane_c == 0, 0xFFFF, -0x10000)
            put("q", 2 * cp, [spread(pltpu.bitcast(t, jnp.int32)) & keep for t in packed])

        def make_q(cp):
            put_q(cp, [pack(t) for t in x_matmul("wq", cp)])

        def score_tiles(hq, odd, base, dh):
            q = [load("q", (3 * hq) >> 1, i) for i in range(2)]
            out = []
            for b in range(NB):
                for t in range(NA // 8):
                    r = tile_matmul(q[(odd + t) // 2],
                                    [load("k", base, dh * HV + (8 * t + a) * NB + b)
                                     for a in range(8)])
                    out.append(r[8:16] if (odd + t) % 2 else r[0:8])
            return out

        def rows_of(v):
            return jnp.broadcast_to(v, (8, 128))

        def lane_softmax(raw, slot):
            parts = []
            for b in range(NB):
                r = total(raw(b))
                if b % 4:
                    parts[-1] = jnp.where((sub >> 1) == b % 4, r, parts[-1])
                else:
                    parts.append(r)
                if b % 2:
                    yield
            top = jnp.max(functools.reduce(jnp.maximum, parts), axis=0, keepdims=True)
            top = rows_of(jnp.maximum(top, LOWEST))
            yield
            yield
            e = [jnp.exp((s - top) * SCALE) for s in parts]
            yield
            yield
            put(f"stat{slot}", 0, [top, rows_of(jnp.sum(total(e), axis=0, keepdims=True))])
            for i in range(2 * NB):
                put(f"p{slot}", i, [rows_of(e[i // 8][i % 8:i % 8 + 1])])
                if i % 4 == 3:
                    yield

        def put_lane_softmax(raw, slot):
            for _ in lane_softmax(lambda b: raw[3 * b:3 * b + 3], slot):
                pass

        def put_lane_weights(slot):
            top, part = get(f"stat{slot}", 0, 2)
            w = jnp.exp((top - jnp.max(top, axis=1, keepdims=True)) * SCALE)
            w = w.astype(BF16).astype(F32)
            put(f"den{slot}", 0, [w * part])
            put("w", slot, [w])

        def put_inverse(slot):
            den = jnp.sum(get(f"den{slot}", 0, 1)[0], axis=1, keepdims=True)
            put("inv", slot, [rows_of(1.0 / den)])

        def p_times_v(base, slot, out, side=None):
            for a0 in range(0, NA, ACC):
                acc = [None] * ACC
                for b in range(NB):
                    p0, p1 = get(f"p{slot}", 0, 2, 2 * b)
                    for i in range(ACC):
                        v = load("v", base, (a0 + i) * NB + b)
                        v = pltpu.bitcast(v, BF16).astype(F32)
                        t = v[0:8] * p0
                        acc[i] = (acc[i] + t if b else t) + v[8:16] * p1
                    if side is not None and (b + 1) * ACC % 8 == 0:
                        next(side, None)
                out[slot * DH + a0 * 8:slot * DH + (a0 + ACC) * 8] = jnp.concatenate(acc, axis=0)

        def retile(name, k0, n):
            def body(k, _):
                base = k * KT
                for g in range(8):
                    old = [load(name, base, g * ND + t) for t in range(ND)]
                    half = [part for v in old for part in (v[0:4], v[4:8])]
                    for t in range(ND):
                        buf[base + (at[name] + g * ND + t)] = jnp.concatenate(
                            [half[t], half[ND + t]], axis=0)
            if n == 1:
                body(k0, None)
            else:
                lax.fori_loop(k0, k0 + n, body, None)

        def row_tiles(lhs, name, base, k):
            return [tile_matmul(lhs, [load(name, base, k * KT + g * ND + t)
                                      for g in range(8)]) for t in range(ND)]

        def add_rows(y, raw):
            return [total(([] if y is None else [y[t]]) + raw[t::ND]) for t in range(ND)]

        def merge_lanes():
            w = get("w", 0, 2)
            out = []
            for j, heads in enumerate((w[:1], w, w[1:])):
                r = lax.dot_general(jnp.concatenate(heads, axis=0), pv[128 * j:128 * j + 128],
                                    (((1,), (1,)), ((), ())), preferred_element_type=F32)
                out += jnp.split(r, len(heads))
            return out

        def head_outputs(raw):
            r0, r1 = get("inv", 0, 2)
            return [raw[0] * r0, jnp.where(lane < DH - 128, raw[1] * r0, raw[2] * r1),
                    raw[3] * r1]

        def out_tiles(lhs, pair):
            base = pair * (3 * KT)
            return [t for j in range(3) for t in row_tiles(lhs[j], "wo", base, j)]

        def residual(x, y):
            y = jnp.concatenate(y, axis=1)
            return (x + y.astype(BF16).astype(F32)).astype(BF16).astype(F32)

        def glu_hidden(g, u):
            return jax.nn.sigmoid(g) * u

        zeros = [jnp.zeros((8, 128), F32)] * ND

        start_wq(0, S_Q)
        x_copy = pltpu.make_async_copy(x_hbm, xb, sems.at[S_X])
        x_copy.start()
        start_wq(1, S_Q + 1)
        put("spread", 0, [((sub >> 2) << 6) | ((lane >> 4) << 3) | (lane & 7)])
        x_copy.wait()
        x = jnp.broadcast_to(xb[...].astype(F32), (8, d_model))
        layernorm_lhs(x)
        put("y", 0, zeros)
        for s in range(NSQ):
            wait_wq(s, S_Q + s % 2)
            if s + 2 < NSQ:
                start_wq(s + 2, S_Q + s % 2)
            elif s + 2 == NSQ:
                start_head("k", 0, S_K)
            else:
                start_head("v", 0, S_V)

        def head1(h, _):
            odd = h & 1
            pair = h >> 1

            @pl.when(h < NQ // 2)
            def _():
                make_q(h)

            wait("k", h * HV, HV, S_K)

            @pl.when(h + 1 < HQ)
            def _():
                start_head("k", h + 1, S_K)

            @pl.when(h + 1 == HQ)
            def _():
                start("wg", 0, sizes["wg"], S_G)

            for slot in range(2):
                @pl.when(odd == slot)
                def _():
                    put_lane_softmax(score_tiles(h, slot, h * HV, 0), slot)
                    put_lane_weights(slot)
                    put_inverse(slot)

            wait("v", h * HV, HV, S_V)

            @pl.when(h + 1 < HQ)
            def _():
                start_head("v", h + 1, S_V)

            @pl.when(h + 1 == HQ)
            def _():
                start("wu", 0, sizes["wu"], S_U)

            @pl.when(odd == 0)
            def _():
                start("wo", pair * (3 * KT), 3 * KT, S_O)
                p_times_v(h * HV, 0, pv)

            @pl.when(odd == 1)
            def _():
                p_times_v(h * HV, 1, pv)
                wait("wo", pair * (3 * KT), 3 * KT, S_O)
                retile("wo", 3 * pair, 3)
                lhs = head_outputs(merge_lanes())
                put("y", 0, add_rows(get("y", 0, ND), out_tiles(lhs, pair)))

        lax.fori_loop(0, HQ, head1, None)

        for i, (k0, k1) in enumerate(WD_PIECES):
            start("wd", k0 * KT, (k1 - k0) * KT, S_D + i)
        x = residual(x, get("y", 0, ND))
        layernorm_lhs(x)
        wait("wg", 0, sizes["wg"], S_G)
        gate = [t for cp in range(NF // 2) for t in x_matmul("wg", cp)]
        wait("wu", 0, sizes["wu"], S_U)
        up = [t for cp in range(NF // 2) for t in x_matmul("wu", cp)]
        hid = [glu_hidden(g, u) for g, u in zip(gate, up)]
        y = None
        for i, (k0, k1) in enumerate(WD_PIECES):
            wait("wd", k0 * KT, (k1 - k0) * KT, S_D + i)
            retile("wd", k0, k1 - k0)
            for k in range(k0, k1):
                y = add_rows(y, row_tiles(hid[k], "wd", 0, k))
        x = residual(x, y)

        layernorm_lhs(x)
        for cp in range(3):
            make_q(cp)
        put("raw_q", 0, [t for cp in (3, 4) for t in x_tiles("wq", cp)])
        put_lane_softmax(score_tiles(0, 0, 0, 0), 0)
        put("raw_s1", 0, score_tiles(1, 1, 0, 1))
        put("y", 0, zeros)
        put("o", 0, zeros[:3])

        def pair2(more_q, pair, _):
            def step(slot, side):
                h = 2 * pair + slot
                base = h * HV
                put_lane_weights(slot)
                put_inverse(1 - slot)
                scores = lambda b: get(f"raw_s{1 - slot}", 0, 3, 3 * b)
                p_times_v(base, slot, pv if slot else pv_new,
                          itertools.chain(lane_softmax(scores, 1 - slot), side))
                put(f"raw_s{slot}", 0,
                    score_tiles(jnp.minimum(h + 2, HQ - 2 + slot), slot, base, 2))

            def even():
                def side():
                    for i, off in enumerate((0, 1, 4 * ND, 4 * ND + 1)):
                        t = total([get("raw_q", 0, 1, off + 2 * k)[0] for k in range(2 * ND)])
                        put("q_sum", i, [pack(t * get("rstd", 0, 1)[0])])
                        yield

                put("raw_o", 0, merge_lanes())
                step(0, side())
                put("raw_y", 0, out_tiles(get("o", 0, 3),
                                          jnp.maximum(pair - 2, 0)))

            def odd():
                h = 2 * pair + 1

                def side():
                    pv[0:DH] = pv_new[...]
                    yield
                    y = get("y", 0, ND)
                    for t in range(ND):
                        new = total([get("raw_y", 0, 1, j * ND + t)[0] for j in range(3)])
                        put("y", t, [y[t] + jnp.where(pair > 1, new, 0.0)])
                        yield

                put("o", 0, head_outputs(get("raw_o", 0, 4)))
                step(1, side())
                for i in range(2):
                    put_q(jnp.minimum(h + 2 + i, NQ // 2 - 1), get("q_sum", 0, 2, 2 * i))
                if more_q:
                    put("raw_q", 0, [t for i in range(2) for t in x_tiles(
                        "wq", jnp.minimum(h + 4 + i, NQ // 2 - 1))])

            even()
            pl.when(pair >> 8 == 0)(odd)

        q_done = (NQ // 2 - 4) // 2
        lax.fori_loop(0, q_done, functools.partial(pair2, True), None)
        lax.fori_loop(q_done, HQ // 2, functools.partial(pair2, False), None)
        put_inverse(1)
        raw = merge_lanes()
        y = add_rows(get("y", 0, ND),
                     out_tiles(get("o", 0, 3), HQ // 2 - 2))
        x = residual(x, add_rows(y, out_tiles(head_outputs(raw), HQ // 2 - 1)))

        layernorm_lhs(x)
        y, hid = None, []
        for cp in range(NF // 2 + GLU_LAG):
            if cp < NF // 2:
                hid += map(glu_hidden, x_matmul("wg", cp), x_matmul("wu", cp))
            for k in range(2 * (cp - GLU_LAG), 2 * (cp - GLU_LAG + 1)):
                if k >= 0:
                    y = add_rows(y, row_tiles(hid[k], "wd", 0, k))
        o_ref[...] = residual(x, y)[0:1].astype(o_ref.dtype)

    scratch = [
        pltpu.VMEM((1, d_model), BF16),
        pltpu.VMEM((n_vregs, 8, 128), U32),
        pltpu.VMEM((NQ // 2, 2 * KT, 8, 128), U32),
        pltpu.VMEM((2 * DH, 128), F32),
        pltpu.VMEM((DH, 128), F32),
        pltpu.SemaphoreType.DMA((n_sems,)),
    ] + [pltpu.VMEM((n, 8, 128), U32) for n in work.values()]
    return kernel, scratch


@jax.jit
def pallas_interleave_layers__sliding_block_cached__glu_gated_glu__decode_kernel(
    A_x: jax.Array,
    A_k_cache: jax.Array,
    A_v_cache: jax.Array,
    A_wq: jax.Array,
    A_wo: jax.Array,
    B_x: jax.Array,
    B_w_gate: jax.Array,
    B_w_up: jax.Array,
    B_w_down: jax.Array,
):
    del B_x
    d_model, d_ff = B_w_gate.shape
    sk = A_k_cache.shape[2]
    win = min(4096, max(256, sk // 4))
    assert A_x.shape == (1, 1, 640) and d_ff == 1536 and win == 4096
    assert A_k_cache.shape == A_v_cache.shape == (1, HQ, sk, DH) and sk % 256 == 0

    def cache_view(c):
        return _vreg_view(jnp.swapaxes(c, 2, 3).reshape(HQ, DH, sk))

    kernel, scratch = _make_kernel(d_model, d_ff, sk, win)
    out = pl.pallas_call(
        kernel,
        out_shape=jax.ShapeDtypeStruct((1, d_model), A_x.dtype),
        in_specs=[pl.BlockSpec(memory_space=pl.ANY)] * 8,
        out_specs=pl.BlockSpec(memory_space=pltpu.VMEM),
        scratch_shapes=scratch,
        compiler_params=pltpu.CompilerParams(vmem_limit_bytes=126 * 1024 * 1024,
                                             disable_bounds_checks=True),
        name="attn_glu_x2",
    )(A_x.reshape(1, d_model), cache_view(A_k_cache), cache_view(A_v_cache),
      *map(_vreg_view, (A_wq, A_wo, B_w_gate, B_w_up, B_w_down)))
    return out.reshape(A_x.shape)
```

```python
import functools
import itertools

import jax
import jax.numpy as jnp
from jax import lax
import jax.experimental.pallas as pl
import jax.experimental.pallas.tpu as pltpu

F32 = jnp.float32
BF16 = jnp.bfloat16
U32 = jnp.uint32

HQ, DH = 32, 192
NA = DH // 8
CH = 4
EPS = 1e-5
SCALE = DH ** -0.5
LOWEST = -3e38
WD_PIECES = ((0, 6), (6, 9), (9, 11), (11, 12))
ACC = 8
GLU_LAG = 2


def _vreg_view(w):
    *lead, r, c = w.shape
    n = len(lead)
    t = w.reshape(*lead, r // 8, 8, c // 128, 128)
    t = jnp.transpose(t, (*range(n), n, n + 2, n + 1, n + 3))
    return t.reshape(-1, 16, 128)


def _make_kernel(d_model, d_ff, sk, win):
    NB = win // 256
    HV = NA * NB
    ND = d_model // 128
    NF = d_ff // 128
    NQ = HQ * DH // 128
    KT = 8 * ND
    NSQ = 3
    qn = NQ // 2 // NSQ
    S_K, S_V, S_O, S_Q = 0, 1, 2, 3
    S_G, S_U, S_X, S_D = S_K, S_V, S_O, S_Q
    n_sems = S_D + max(2, len(WD_PIECES))
    sizes = dict(k=HQ * HV, v=HQ * HV, wo=NQ * KT, wg=NF * KT, wu=NF * KT, wd=NF * KT)
    work = dict(x=2 * ND, rstd=1, spread=1, q=NQ, q_sum=4, p0=2 * NB, p1=2 * NB, stat0=2,
                stat1=2, w=2, den0=1, den1=1, inv=2, o=3, y=ND,
                raw_s0=3 * NB, raw_s1=3 * NB, raw_q=8 * ND, raw_o=4, raw_y=3 * ND)
    at, n_vregs = {}, 0
    for name, size in sizes.items():
        at[name], n_vregs = n_vregs, n_vregs + size

    def kernel(x_hbm, k_hbm, v_hbm, wq_hbm, wo_hbm, wg_hbm, wu_hbm, wd_hbm, o_ref,
               xb, buf, wq, pv, pv_new, sems, *work_refs):
        wk = dict(zip(work, work_refs))
        lane = lax.broadcasted_iota(jnp.int32, (8, 128), 1)
        sub = lax.broadcasted_iota(jnp.int32, (8, 128), 0)
        lane_c = (lane >> 3) & 1

        hbm = dict(k=k_hbm, v=v_hbm, wq=wq_hbm, wo=wo_hbm, wg=wg_hbm, wu=wu_hbm, wd=wd_hbm)
        hbm = {name: ref.bitcast(U32) for name, ref in hbm.items()}

        def streams(name, src, src_stride, dst, dst_stride, count, sem):
            def body(c, _):
                for i in range(count):
                    pltpu.make_async_copy(
                        hbm[name].at[pl.ds(src + c * CH + i * src_stride, CH)],
                        buf.at[pl.ds(dst + c * CH + (at[name] + i * dst_stride), CH)],
                        sems.at[sem]).start(priority=i % 2)
            lax.fori_loop(0, dst_stride // CH, body, None)

        def start(name, i0, n, sem):
            count = 6 if n % (6 * CH) == 0 else 2
            streams(name, i0, n // count, i0, n // count, count, sem)

        def start_head(name, h, sem):
            row = sk // 256
            streams(name, h * (NA * row) + (row - NB), row, h * HV, NB, NA, sem)

        def start_wq(step, sem):
            part = 2 * KT // 4

            def body(j, _):
                for cp in range(step * qn, (step + 1) * qn, CH):
                    for i in range(4):
                        a = j + i * part
                        pltpu.make_async_copy(hbm["wq"].at[pl.ds(a * (NQ // 2) + cp, CH)],
                                              wq.at[pl.ds(cp, CH), a],
                                              sems.at[sem]).start(priority=i % 2)
            lax.fori_loop(0, part, body, None)

        def wait_wq(step, sem):
            blk = wq.at[pl.ds(step * qn, qn)]
            pltpu.make_async_copy(blk, blk, sems.at[sem]).wait()

        def wait(name, i0, n, sem):
            blk = buf.at[pl.ds(at[name] + i0, n)]
            pltpu.make_async_copy(blk, blk, sems.at[sem]).wait()

        def load(name, base, off):
            return buf[base + (at[name] + off)] if name in sizes else wk[name][base + off]

        def put(name, base, vals):
            for i, v in enumerate(vals):
                wk[name][base + i] = pltpu.bitcast(v, U32)

        def get(name, base, n, off=0):
            return [pltpu.bitcast(load(name, base, off + i), F32) for i in range(n)]

        def tile_matmul(lhs, rhs):
            if lhs.dtype != F32:
                lhs = pltpu.bitcast(lhs, BF16)
            return lax.dot_general(lhs, pltpu.bitcast(jnp.concatenate(rhs, axis=0), BF16),
                                   (((1,), (0,)), ((), ())), preferred_element_type=F32)

        def pack(top, bottom=None):
            bottom = top if bottom is None else bottom
            return pltpu.bitcast(jnp.concatenate([top, bottom], axis=0).astype(BF16), U32)

        def spread(t):
            idx = pltpu.bitcast(load("spread", 0, 0), jnp.int32)
            return jnp.take_along_axis(t, idx, axis=1, mode="promise_in_bounds",
                                       wrap_negative_indices=False)

        def layernorm_lhs(x):
            m = jnp.sum(x, axis=1, keepdims=True) * (1.0 / d_model)
            xc = x - m
            v = jnp.sum(xc * xc, axis=1, keepdims=True) * (1.0 / d_model)
            put("rstd", 0, [rows_of(lax.rsqrt(v + EPS))])
            out = []
            for t in range(ND):
                both = spread(x[:, t * 128:(t + 1) * 128]) - m
                for half in range(2):
                    n = rows_of(both[4 * half:4 * half + 1])
                    out.append(pack(*(jnp.where(lane_c == c, n, 0.0) for c in range(2))))
            put("x", 0, out)

        def total(vals):
            return functools.reduce(jnp.add, vals)

        def x_tiles(name, cp):
            out = []
            for i in range(2 * ND):
                rhs = [wq[cp, a] if name == "wq" else load(name, cp, a * (NF // 2))
                       for a in range(8 * i, 8 * i + 8)]
                r = tile_matmul(load("x", 0, i), rhs)
                out += [r[0:8], r[8:16]]
            return out

        def x_matmul(name, cp):
            raw = x_tiles(name, cp)
            rstd, = get("rstd", 0, 1)
            return total(raw[0::2]) * rstd, total(raw[1::2]) * rstd

        def put_q(cp, packed):
            keep = jnp.where(lane_c == 0, 0xFFFF, -0x10000)
            put("q", 2 * cp, [spread(pltpu.bitcast(t, jnp.int32)) & keep for t in packed])

        def make_q(cp):
            put_q(cp, [pack(t) for t in x_matmul("wq", cp)])

        def score_tiles(hq, odd, base, dh):
            q = [load("q", (3 * hq) >> 1, i) for i in range(2)]
            out = []
            for b in range(NB):
                for t in range(NA // 8):
                    r = tile_matmul(q[(odd + t) // 2],
                                    [load("k", base, dh * HV + (8 * t + a) * NB + b)
                                     for a in range(8)])
                    out.append(r[8:16] if (odd + t) % 2 else r[0:8])
            return out

        def rows_of(v):
            return jnp.broadcast_to(v, (8, 128))

        def lane_softmax(raw, slot):
            parts = []
            for b in range(NB):
                r = total(raw(b))
                if b % 4:
                    parts[-1] = jnp.where((sub >> 1) == b % 4, r, parts[-1])
                else:
                    parts.append(r)
                if b % 2:
                    yield
            top = jnp.max(functools.reduce(jnp.maximum, parts), axis=0, keepdims=True)
            top = rows_of(jnp.maximum(top, LOWEST))
            yield
            yield
            e = [jnp.exp((s - top) * SCALE) for s in parts]
            yield
            yield
            put(f"stat{slot}", 0, [top, rows_of(jnp.sum(total(e), axis=0, keepdims=True))])
            for i in range(2 * NB):
                put(f"p{slot}", i, [rows_of(e[i // 8][i % 8:i % 8 + 1])])
                if i % 4 == 3:
                    yield

        def put_lane_softmax(raw, slot):
            for _ in lane_softmax(lambda b: raw[3 * b:3 * b + 3], slot):
                pass

        def put_lane_weights(slot):
            top, part = get(f"stat{slot}", 0, 2)
            w = jnp.exp((top - jnp.max(top, axis=1, keepdims=True)) * SCALE)
            w = w.astype(BF16).astype(F32)
            put(f"den{slot}", 0, [w * part])
            put("w", slot, [w])

        def put_inverse(slot):
            den = jnp.sum(get(f"den{slot}", 0, 1)[0], axis=1, keepdims=True)
            put("inv", slot, [rows_of(1.0 / den)])

        def p_times_v(base, slot, out, side=None):
            for a0 in range(0, NA, ACC):
                acc = [None] * ACC
                for b in range(NB):
                    p0, p1 = get(f"p{slot}", 0, 2, 2 * b)
                    for i in range(ACC):
                        v = load("v", base, (a0 + i) * NB + b)
                        v = pltpu.bitcast(v, BF16).astype(F32)
                        t = v[0:8] * p0
                        acc[i] = (acc[i] + t if b else t) + v[8:16] * p1
                    if side is not None and (b + 1) * ACC % 8 == 0:
                        next(side, None)
                out[slot * DH + a0 * 8:slot * DH + (a0 + ACC) * 8] = jnp.concatenate(acc, axis=0)

        def retile(name, k0, n):
            def body(k, _):
                base = k * KT
                for g in range(8):
                    old = [load(name, base, g * ND + t) for t in range(ND)]
                    half = [part for v in old for part in (v[0:4], v[4:8])]
                    for t in range(ND):
                        buf[base + (at[name] + g * ND + t)] = jnp.concatenate(
                            [half[t], half[ND + t]], axis=0)
            if n == 1:
                body(k0, None)
            else:
                lax.fori_loop(k0, k0 + n, body, None)

        def row_tiles(lhs, name, base, k):
            return [tile_matmul(lhs, [load(name, base, k * KT + g * ND + t)
                                      for g in range(8)]) for t in range(ND)]

        def add_rows(y, raw):
            return [total(([] if y is None else [y[t]]) + raw[t::ND]) for t in range(ND)]

        def merge_lanes():
            w = get("w", 0, 2)
            out = []
            for j, heads in enumerate((w[:1], w, w[1:])):
                r = lax.dot_general(jnp.concatenate(heads, axis=0), pv[128 * j:128 * j + 128],
                                    (((1,), (1,)), ((), ())), preferred_element_type=F32)
                out += jnp.split(r, len(heads))
            return out

        def head_outputs(raw):
            r0, r1 = get("inv", 0, 2)
            return [raw[0] * r0, jnp.where(lane < DH - 128, raw[1] * r0, raw[2] * r1),
                    raw[3] * r1]

        def out_tiles(lhs, pair):
            base = pair * (3 * KT)
            return [t for j in range(3) for t in row_tiles(lhs[j], "wo", base, j)]

        def residual(x, y):
            y = jnp.concatenate(y, axis=1)
            return (x + y.astype(BF16).astype(F32)).astype(BF16).astype(F32)

        def glu_hidden(g, u):
            return jax.nn.sigmoid(g) * u

        zeros = [jnp.zeros((8, 128), F32)] * ND

        start_wq(0, S_Q)
        x_copy = pltpu.make_async_copy(x_hbm, xb, sems.at[S_X])
        x_copy.start()
        start_wq(1, S_Q + 1)
        put("spread", 0, [((sub >> 2) << 6) | ((lane >> 4) << 3) | (lane & 7)])
        x_copy.wait()
        x = jnp.broadcast_to(xb[...].astype(F32), (8, d_model))
        layernorm_lhs(x)
        put("y", 0, zeros)
        for s in range(NSQ):
            wait_wq(s, S_Q + s % 2)
            if s + 2 < NSQ:
                start_wq(s + 2, S_Q + s % 2)
            elif s + 2 == NSQ:
                start_head("k", 0, S_K)
            else:
                start_head("v", 0, S_V)

        def head1(h, _):
            odd = h & 1
            pair = h >> 1

            @pl.when(h < NQ // 2)
            def _():
                make_q(h)

            wait("k", h * HV, HV, S_K)

            @pl.when(h + 1 < HQ)
            def _():
                start_head("k", h + 1, S_K)

            @pl.when(h + 1 == HQ)
            def _():
                start("wg", 0, sizes["wg"], S_G)

            for slot in range(2):
                @pl.when(odd == slot)
                def _():
                    put_lane_softmax(score_tiles(h, slot, h * HV, 0), slot)
                    put_lane_weights(slot)
                    put_inverse(slot)

            wait("v", h * HV, HV, S_V)

            @pl.when(h + 1 < HQ)
            def _():
                start_head("v", h + 1, S_V)

            @pl.when(h + 1 == HQ)
            def _():
                start("wu", 0, sizes["wu"], S_U)

            @pl.when(odd == 0)
            def _():
                start("wo", pair * (3 * KT), 3 * KT, S_O)
                p_times_v(h * HV, 0, pv)

            @pl.when(odd == 1)
            def _():
                p_times_v(h * HV, 1, pv)
                wait("wo", pair * (3 * KT), 3 * KT, S_O)
                retile("wo", 3 * pair, 3)
                lhs = head_outputs(merge_lanes())
                put("y", 0, add_rows(get("y", 0, ND), out_tiles(lhs, pair)))

        lax.fori_loop(0, HQ, head1, None)

        for i, (k0, k1) in enumerate(WD_PIECES):
            start("wd", k0 * KT, (k1 - k0) * KT, S_D + i)
        x = residual(x, get("y", 0, ND))
        layernorm_lhs(x)
        wait("wg", 0, sizes["wg"], S_G)
        gate = [t for cp in range(NF // 2) for t in x_matmul("wg", cp)]
        wait("wu", 0, sizes["wu"], S_U)
        up = [t for cp in range(NF // 2) for t in x_matmul("wu", cp)]
        hid = [glu_hidden(g, u) for g, u in zip(gate, up)]
        y = None
        for i, (k0, k1) in enumerate(WD_PIECES):
            wait("wd", k0 * KT, (k1 - k0) * KT, S_D + i)
            retile("wd", k0, k1 - k0)
            for k in range(k0, k1):
                y = add_rows(y, row_tiles(hid[k], "wd", 0, k))
        x = residual(x, y)

        layernorm_lhs(x)
        for cp in range(3):
            make_q(cp)
        put("raw_q", 0, [t for cp in (3, 4) for t in x_tiles("wq", cp)])
        put_lane_softmax(score_tiles(0, 0, 0, 0), 0)
        put("raw_s1", 0, score_tiles(1, 1, 0, 1))
        put("y", 0, zeros)
        put("o", 0, zeros[:3])

        def pair2(more_q, pair, _):
            def step(slot, side):
                h = 2 * pair + slot
                base = h * HV
                put_lane_weights(slot)
                put_inverse(1 - slot)
                scores = lambda b: get(f"raw_s{1 - slot}", 0, 3, 3 * b)
                p_times_v(base, slot, pv if slot else pv_new,
                          itertools.chain(lane_softmax(scores, 1 - slot), side))
                put(f"raw_s{slot}", 0,
                    score_tiles(jnp.minimum(h + 2, HQ - 2 + slot), slot, base, 2))

            def even():
                def side():
                    for i, off in enumerate((0, 1, 4 * ND, 4 * ND + 1)):
                        t = total([get("raw_q", 0, 1, off + 2 * k)[0] for k in range(2 * ND)])
                        put("q_sum", i, [pack(t * get("rstd", 0, 1)[0])])
                        yield

                put("raw_o", 0, merge_lanes())
                step(0, side())
                put("raw_y", 0, out_tiles(get("o", 0, 3), jnp.maximum(pair - 2, 0)))

            def odd():
                h = 2 * pair + 1

                def side():
                    pv[0:DH] = pv_new[...]
                    yield
                    y = get("y", 0, ND)
                    for t in range(ND):
                        new = total([get("raw_y", 0, 1, j * ND + t)[0] for j in range(3)])
                        put("y", t, [y[t] + jnp.where(pair > 1, new, 0.0)])
                        yield

                put("o", 0, head_outputs(get("raw_o", 0, 4)))
                step(1, side())
                for i in range(2):
                    put_q(jnp.minimum(h + 2 + i, NQ // 2 - 1), get("q_sum", 0, 2, 2 * i))
                if more_q:
                    put("raw_q", 0, [t for i in range(2) for t in x_tiles(
                        "wq", jnp.minimum(h + 4 + i, NQ // 2 - 1))])

            even()
            pl.when(pair >> 8 == 0)(odd)

        q_done = (NQ // 2 - 4) // 2
        lax.fori_loop(0, q_done, functools.partial(pair2, True), None)
        lax.fori_loop(q_done, HQ // 2, functools.partial(pair2, False), None)
        put_inverse(1)
        raw = merge_lanes()
        y = add_rows(get("y", 0, ND), out_tiles(get("o", 0, 3), HQ // 2 - 2))
        x = residual(x, add_rows(y, out_tiles(head_outputs(raw), HQ // 2 - 1)))

        layernorm_lhs(x)
        y, hid = None, []
        for cp in range(NF // 2 + GLU_LAG):
            if cp < NF // 2:
                hid += map(glu_hidden, x_matmul("wg", cp), x_matmul("wu", cp))
            for k in range(2 * (cp - GLU_LAG), 2 * (cp - GLU_LAG + 1)):
                if k >= 0:
                    y = add_rows(y, row_tiles(hid[k], "wd", 0, k))
        o_ref[...] = residual(x, y)[0:1].astype(o_ref.dtype)

    scratch = [
        pltpu.VMEM((1, d_model), BF16),
        pltpu.VMEM((n_vregs, 8, 128), U32),
        pltpu.VMEM((NQ // 2, 2 * KT, 8, 128), U32),
        pltpu.VMEM((2 * DH, 128), F32),
        pltpu.VMEM((DH, 128), F32),
        pltpu.SemaphoreType.DMA((n_sems,)),
    ] + [pltpu.VMEM((n, 8, 128), U32) for n in work.values()]
    return kernel, scratch


@jax.jit
def pallas_interleave_layers__sliding_block_cached__glu_gated_glu__decode_kernel(
    A_x: jax.Array,
    A_k_cache: jax.Array,
    A_v_cache: jax.Array,
    A_wq: jax.Array,
    A_wo: jax.Array,
    B_x: jax.Array,
    B_w_gate: jax.Array,
    B_w_up: jax.Array,
    B_w_down: jax.Array,
):
    del B_x
    d_model, d_ff = B_w_gate.shape
    sk = A_k_cache.shape[2]
    win = min(4096, max(256, sk // 4))
    assert A_x.shape == (1, 1, 640) and d_ff == 1536 and win == 4096
    assert A_k_cache.shape == A_v_cache.shape == (1, HQ, sk, DH) and sk % 256 == 0

    def cache_view(c):
        return _vreg_view(jnp.swapaxes(c, 2, 3).reshape(HQ, DH, sk))

    kernel, scratch = _make_kernel(d_model, d_ff, sk, win)
    out = pl.pallas_call(
        kernel,
        out_shape=jax.ShapeDtypeStruct((1, d_model), A_x.dtype),
        in_specs=[pl.BlockSpec(memory_space=pl.ANY)] * 8,
        out_specs=pl.BlockSpec(memory_space=pltpu.VMEM),
        scratch_shapes=scratch,
        compiler_params=pltpu.CompilerParams(vmem_limit_bytes=126 * 1024 * 1024,
                                             disable_bounds_checks=True),
        name="attn_glu_x2",
    )(A_x.reshape(1, d_model), cache_view(A_k_cache), cache_view(A_v_cache),
      *map(_vreg_view, (A_wq, A_wo, B_w_gate, B_w_up, B_w_down)))
    return out.reshape(A_x.shape)
```
